```python
import jax
import jax.numpy as jnp

def _softmax(x, axis=-1):
    return jax.nn.softmax(x, axis=axis)
def _gelu(x):
    return jax.nn.gelu(x, approximate=True)
def _silu(x):
    return jax.nn.silu(x)
def _sigmoid(x):
    return jax.nn.sigmoid(x)
def _layernorm(x, axis=-1, eps=1e-5):
    m = jnp.mean(x, axis=axis, keepdims=True)
    v = jnp.var(x, axis=axis, keepdims=True)
    return (x - m) / jnp.sqrt(v + eps)
def _scatter_add(tgt, idx, src, axis=0):
    return tgt.at[idx].add(src)
def _segment_sum(src, seg, n):
    return jax.ops.segment_sum(src, seg, n)
class _Rng:
    def __init__(self, key):
        self._k = key
    def _next(self):
        self._k, sub = jax.random.split(self._k)
        return sub
    def normal(self, shape):
        return jax.random.normal(self._next(), shape, dtype=jnp.bfloat16)
    def randint(self, lo, hi, shape):
        return jax.random.randint(self._next(), shape, lo, hi, dtype=jnp.int32)
    def uniform(self, shape, lo=0.0, hi=1.0):
        return jax.random.uniform(self._next(), shape, jnp.bfloat16, lo, hi)
    def permutation(self, n):
        return jax.random.permutation(self._next(), n)


kernel_name = 'sequential_preLN__sliding_local_dilated__glu_gated_geglu__prompt'

def setup_inputs():
    _rng = _Rng(jax.random.key(int.from_bytes(__import__("os").urandom(4), "little")))
    _w = (lambda a: (lambda t: t.astype(jnp.bfloat16) if jnp.issubdtype(t.dtype, jnp.floating) else t)(jnp.asarray(a)))
    def _A_setup():
        B, S, D = 1, 2048, 1024
        return {
            "x": _w((lambda *s: _rng.normal(s) * 0.05)(B, S, D)),
            "wqkv": _w((lambda *s: _rng.normal(s) * 0.05)(D, 3 * D)),
            "wo": _w((lambda *s: _rng.normal(s) * 0.05)(D, D)),
        }
    _A_in = _A_setup()

    def _B_setup():
        B, S, Dm, Df = 1, 2048, 1024, 3584
        return {
            "x": _w((lambda *s: _rng.normal(s) * 0.05)(B, S, Dm)),
            "w_gate": _w((lambda *s: _rng.normal(s) * 0.05)(Dm, Df) * (Dm ** -0.5)),
            "w_up": _w((lambda *s: _rng.normal(s) * 0.05)(Dm, Df) * (Dm ** -0.5)),
            "w_down": _w((lambda *s: _rng.normal(s) * 0.05)(Df, Dm) * (Df ** -0.5)),
        }
    _B_in = _B_setup()

    return {
        "A_x": _A_in["x"],
        "A_wqkv": _A_in["wqkv"],
        "A_wo": _A_in["wo"],
        "B_x": _B_in["x"],
        "B_w_gate": _B_in["w_gate"],
        "B_w_up": _B_in["w_up"],
        "B_w_down": _B_in["w_down"],
    }

def reference(A_x, A_wqkv, A_wo, B_x, B_w_gate, B_w_up, B_w_down):
    def _A_ref(x, wqkv, wo):
        B, S, D = x.shape
        H = 32; Dh = D // H
        W, dil = 8, 2
        qkv = (lambda x, *d: x.transpose(*d))((x @ wqkv).reshape(B, S, 3, H, Dh), 2, 0, 3, 1, 4)
        q, k, v = qkv[0], qkv[1], qkv[2]
        scale = Dh ** -0.5
        pos = jnp.arange(S)
        off = jnp.arange(W) * dil
        idx = pos[:, None] - off[None, :]
        mask = idx >= 0
        idx_c = jnp.where(mask, idx, 0).reshape(-1)
        kg = k[:, :, idx_c, :].reshape(B, H, S, W, Dh)
        vg = v[:, :, idx_c, :].reshape(B, H, S, W, Dh)
        logits = jnp.einsum("bhsd,bhswd->bhsw", q, kg) * scale
        logits = jnp.where(mask[None, None, :, :], logits, -1e9)
        attn = _softmax(logits, axis=-1)
        o = jnp.einsum("bhsw,bhswd->bhsd", attn, vg)
        return (lambda x, *d: x.transpose(*d))(o, 0, 2, 1, 3).reshape(B, S, D) @ wo

    def _B_ref(x, w_gate, w_up, w_down):
        g = jnp.einsum("bsd,df->bsf", x, w_gate)
        u = jnp.einsum("bsd,df->bsf", x, w_up)
        h = _gelu(g) * u
        return jnp.einsum("bsf,fd->bsd", h, w_down)

    x = A_x
    h = x + _A_ref(_layernorm(x, axis=-1), A_wqkv, A_wo)
    h2 = h + _B_ref(_layernorm(h, axis=-1), B_w_gate, B_w_up, B_w_down)
    return h2
```

```python
import functools
import numpy as np
import jax
import jax.numpy as jnp
from jax import lax
import jax.experimental.pallas as pl
import jax.experimental.pallas.tpu as pltpu

S, D, F = 2048, 1024, 3584
NH, DH, WIN, DIL = 32, 32, 8, 2
HALO = 16
NCB = D // 128
F32, BF16, U32 = jnp.float32, jnp.bfloat16, jnp.uint32
LOG2E = float(np.log2(np.e))
C0 = float(np.sqrt(2.0 / np.pi)); C1 = C0 * 0.044715


def _ln(x):
    m = jnp.mean(x, axis=-1, keepdims=True)
    xc = x - m
    v = jnp.mean(xc * xc, axis=-1, keepdims=True)
    return xc * lax.rsqrt(v + 1e-5)


def _dot(a, b):
    return jnp.dot(a, b, preferred_element_type=F32)


def make(TM=512, FC=512, RG=16, ffn_loop=False, down_whole=True, flags=None):
    NT = S // TM
    NF = F // FC

    def kernel(x_ref, wqkv_hbm, wo_hbm, wg_hbm, wu_hbm, wd_hbm, o_ref,
               wqkv, wo_raw, wo, wg, wu, wd, tmp, qb, kb, vb, ob, hb, hn, ab, sems):
        i = pl.program_id(0)
        cp_qkv = [pltpu.make_async_copy(wqkv_hbm.at[:, pl.ds(j * D, D)], wqkv.at[j], sems.at[j]) for j in range(3)]
        cp_wo = [pltpu.make_async_copy(wo_hbm.at[:, pl.ds(c * 128, 128)], wo_raw.at[c], sems.at[3 + c]) for c in range(NCB)]
        cp_g = pltpu.make_async_copy(wg_hbm, wg, sems.at[11])
        cp_u = pltpu.make_async_copy(wu_hbm, wu, sems.at[12])
        cp_d = pltpu.make_async_copy(wd_hbm, wd, sems.at[13])

        @pl.when(i == 0)
        def _():
            for c in cp_qkv + cp_wo + [cp_g, cp_u, cp_d]:
                c.start()
            for j in range(3):
                cp_qkv[j].wait()

                def body(rb, _):
                    r0 = pl.multiple_of(rb * 256, 256)
                    w = pltpu.bitcast(wqkv[j, pl.ds(r0, 256), :], U32)
                    tmp[...] = w.T
                    p = jnp.concatenate([tmp[pl.ds(d, NH, stride=DH), :] for d in range(DH)], axis=0)
                    wqkv[j, pl.ds(r0, 256), :] = pltpu.bitcast(p.T, BF16)
                lax.fori_loop(0, 4, body, None)
            for c in range(NCB):
                cp_wo[c].wait()
            for c in range(NCB):
                tmp[...] = pltpu.bitcast(wo_raw[c].astype(F32), U32)
                p = jnp.concatenate([tmp[pl.ds(d, NH, stride=DH), :] for d in range(DH)], axis=0)
                wo[:, c * 128:(c + 1) * 128] = pltpu.bitcast(p, F32).astype(BF16)
            kb[:, 0:HALO, :] = jnp.zeros((NCB, HALO, 128), F32)

        @pl.when(i > 0)
        def _():
            kb[:, 0:HALO, :] = kb[:, TM:TM + HALO, :]
            vb[:, 0:HALO, :] = vb[:, TM:TM + HALO, :]

        xn = _ln(x_ref[...].astype(F32)).astype(BF16)
        q = _dot(xn, wqkv[0])
        k = _dot(xn, wqkv[1])
        v = _dot(xn, wqkv[2])
        for c in range(NCB):
            qb[c] = q[:, c * 128:(c + 1) * 128]
            kb[c, HALO:, :] = k[:, c * 128:(c + 1) * 128]
            vb[c, HALO:, :] = v[:, c * 128:(c + 1) * 128]

        @pl.when(i == 0)
        def _():
            for c in range(NCB):
                vb[c, 0:HALO, :] = jnp.broadcast_to(vb[c, HALO:HALO + 1, :], (HALO, 128))

        for g in range(TM // RG):
            r0 = g * RG
            qs = [qb[c, r0:r0 + RG, :] for c in range(NCB)]
            ls = []
            for w in range(WIN):
                a = HALO + r0 - DIL * w
                t = [qs[c] * kb[c, a:a + RG, :] for c in range(NCB)]
                while len(t) > 1:
                    t = [t[n] + t[n + 1] for n in range(0, len(t), 2)]
                l = t[0]
                l = l + pltpu.roll(l, 64, 1)
                l = l + pltpu.roll(l, 32, 1)
                l = l * (DH ** -0.5 * LOG2E)
                if r0 < DIL * w:
                    pos = i * TM + r0 + lax.broadcasted_iota(jnp.int32, (RG, 128), 0)
                    l = jnp.where(pos >= DIL * w, l, -1e9 * LOG2E)
                ls.append(l)
            m = functools.reduce(jnp.maximum, ls)
            ps = [jnp.exp2(l - m) for l in ls]
            inv = 1.0 / functools.reduce(jnp.add, ps)
            ps = [p * inv for p in ps]
            for c in range(NCB):
                t = [ps[w] * vb[c, HALO + r0 - DIL * w:HALO + r0 - DIL * w + RG, :] for w in range(WIN)]
                while len(t) > 1:
                    t = [t[n] + t[n + 1] for n in range(0, len(t), 2)]
                ob[r0:r0 + RG, c * 128:(c + 1) * 128] = t[0].astype(BF16)

        h = x_ref[...].astype(F32) + _dot(ob[...], wo[...])
        hb[...] = h
        hn[...] = _ln(h).astype(BF16)

        @pl.when(i == 0)
        def _():
            cp_g.wait(); cp_u.wait(); cp_d.wait()

        def chunk(c):
            if isinstance(c, int):
                sl = slice(c * FC, (c + 1) * FC)
            else:
                sl = pl.ds(pl.multiple_of(c * FC, FC), FC)
            gg = _dot(hn[...], wg[:, sl])
            uu = _dot(hn[...], wu[:, sl])
            th = jnp.tanh(gg * (gg * gg * C1 + C0))
            a = ((gg * uu) * (th * 0.5 + 0.5)).astype(BF16)
            if down_whole:
                ab[:, sl] = a
            else:
                hb[...] += _dot(a, wd[sl, :])
        if ffn_loop:
            lax.fori_loop(0, NF, lambda c, _: chunk(c), None)
        else:
            for c in range(NF):
                chunk(c)
        if down_whole:
            o_ref[...] = (hb[...] + _dot(ab[...], wd[...])).astype(BF16)
        else:
            o_ref[...] = hb[...].astype(BF16)

    def fn(A_x, A_wqkv, A_wo, B_x, B_w_gate, B_w_up, B_w_down):
        any_spec = pl.BlockSpec(memory_space=pl.ANY)
        out = pl.pallas_call(
            kernel, grid=(NT,),
            in_specs=[pl.BlockSpec((TM, D), lambda i: (i, 0))] + [any_spec] * 5,
            out_specs=pl.BlockSpec((TM, D), lambda i: (i, 0)),
            out_shape=jax.ShapeDtypeStruct((S, D), BF16),
            scratch_shapes=[
                pltpu.VMEM((3, D, D), BF16), pltpu.VMEM((NCB, D, 128), BF16), pltpu.VMEM((D, D), BF16),
                pltpu.VMEM((D, F), BF16), pltpu.VMEM((D, F), BF16), pltpu.VMEM((F, D), BF16),
                pltpu.VMEM((D, 128), U32),
                pltpu.VMEM((NCB, TM, 128), F32), pltpu.VMEM((NCB, HALO + TM, 128), F32), pltpu.VMEM((NCB, HALO + TM, 128), F32),
                pltpu.VMEM((TM, D), BF16), pltpu.VMEM((TM, D), F32), pltpu.VMEM((TM, D), BF16), pltpu.VMEM((TM, F), BF16),
                pltpu.SemaphoreType.DMA((14,)),
            ],
            compiler_params=pltpu.CompilerParams(dimension_semantics=("arbitrary",), vmem_limit_bytes=100 * 2 ** 20, flags=flags),
        )(A_x.reshape(S, D), A_wqkv, A_wo, B_w_gate, B_w_up, B_w_down)
        return out.reshape(1, S, D)
    return fn


_impl = make(512, ffn_loop=True, down_whole=False)


@jax.jit
def pallas_sequential_preLN__sliding_local_dilated__glu_gated_geglu__prompt_kernel(
    A_x, A_wqkv, A_wo, B_x, B_w_gate, B_w_up, B_w_down
):
    return _impl(A_x, A_wqkv, A_wo, B_x, B_w_gate, B_w_up, B_w_down)
```

```python
import functools
import numpy as np
import jax
import jax.numpy as jnp
from jax import lax
import jax.experimental.pallas as pl
import jax.experimental.pallas.tpu as pltpu

S, D, F = 2048, 1024, 3584
NH, DH, WIN, DIL = 32, 32, 8, 2
HALO = 16
NCB = D // 128
PITCH = 33
F32, BF16, U32 = jnp.float32, jnp.bfloat16, jnp.uint32
LOG2E = float(np.log2(np.e))
C0 = float(np.sqrt(2.0 / np.pi)); C1 = C0 * 0.044715
P = functools.partial


def _pk(v):
    return pltpu.bitcast(v.astype(BF16), U32)


def _put(dst, j, row, cols, v):
    if MODE == 0:
        dst[j, _ds(row // 2, 8, 8), cols] = _pk(v)
    else:
        dst.at[j][_ds(row // 2, 8, 8), cols] = _pk(v)


MODE = 1


def _bf(v):
    return pltpu.bitcast(v, BF16)


def _dot(a, b):
    return jnp.dot(a, b, preferred_element_type=F32)


def _lhs7(a11, a12, a21, a22):
    return (a11 + a22, a21 + a22, a11, a22, a11 + a12, a21 - a11, a12 - a22)


def _rhs7(b11, b12, b21, b22):
    f11, f12, f21, f22 = (b.astype(F32) for b in (b11, b12, b21, b22))
    return (f11 + f22, b11, f12 - f22, f21 - f11, b22, f11 + f12, f21 + f22)


def _sum(t):
    return functools.reduce(jnp.add, t)


def _cols(c, n=128):
    return slice(c * n, (c + 1) * n)


def _ds(start, n, align):
    return pl.ds(start if isinstance(start, int) else pl.multiple_of(start, align), n)


def _strassen(prod, emit):
    m1 = prod(0); yield
    m2 = prod(1); c22 = m1 - m2; yield
    m3 = prod(2); c22 = c22 + m3; yield
    m4 = prod(3); c11 = m1 + m4; emit(1, 0, m2 + m4); yield
    m5 = prod(4); c11 = c11 - m5; emit(0, 1, m3 + m5); yield
    emit(1, 1, c22 + prod(5)); yield
    emit(0, 0, c11 + prod(6)); yield


def _weave(main, n, *sides, lead=1):
    done = [0] * len(sides)
    for k in range(n):
        next(main)
        for s, side in enumerate(sides):
            upto = min(len(side), -(-len(side) * (k + 1) // (n - lead)))
            for f in side[done[s]:upto]:
                f()
            done[s] = upto


def make(TM=512, FC=512, PN=128, PM={8:128,9:128,10:128,11:64,12:64,13:128,14:128}, share=False, GN=128, DN=256, L1C={-1: 1, 0: 2, 1: 2, 2: 3.25, 3: 3.5, 4: 3.75, 5: 4},
         PRC={3: .55, 4: 1.05, 5: 1.55, 6: 2.15, 7: 2.75, 8: 3.4, 9: 3.7, 10: 4},
         L2C={13: .6, 14: 1.2, 15: 2.4, 16: 4}, merge=(), unroll=1,
         PVC={9: .5, 10: 1.0, 11: 2.0, 12: 3.0, 13: 3.5, 14: 4}, scopes=False, ahead=2, xfirst=False, upto=16, lead=1, flags={'XLA_TPU_EVENLY_DISTRIBUTE_CRITICAL_NODES': True}, vmem=120, skip=(), only=None):
    NT = S // TM; NF = F // FC; H = TM // 2; FH = FC // 2; DHALF = D // 2
    import contextlib
    scope = jax.named_scope if scopes else (lambda n: contextlib.nullcontext())
    assert NT == 4 and NF % 2 == 1

    def kernel(x_hbm, wqkv_hbm, wo_hbm, wg_hbm, wu_hbm, wd_hbm, o_hbm,
               xb, wraw, wp0, wp1, wp2, wp3, tmp0, tmp1, xa0, xa1, xa2, xa3, ha, qb, pb, kb, vb,
               rg0, ru0, rd0, rg1, ru1, rd1, gu0, dn0, gu1, dn1, sx, sw, sf, so, s0, go, *acc):
        xa = (xa0, xa1, xa2, xa3); hs = tuple(qb.at[:, pl.ds(t * TM, TM)] for t in range(NT))
        wp = (wp0, wp1, wp2, wp3); raw = ((rg0, ru0, rd0), (rg1, ru1, rd1)); fw = ((gu0, dn0), (gu1, dn1))
        cp_x = [pltpu.make_async_copy(x_hbm.at[pl.ds(t * TM, TM)], xb.at[pl.ds(t * TM, TM)], sx.at[t]) for t in range(NT)]
        cp_q = [[pltpu.make_async_copy(wqkv_hbm.at[pl.ds(r, 128), pl.ds(0, D)], wraw.at[0, pl.ds(r, 128)], sw.at[r // 128])
                 for r in (t * 128, DHALF + t * 128)] for t in range(4)]
        cp_w = {1: pltpu.make_async_copy(wqkv_hbm.at[:, pl.ds(D, D)], wraw.at[1], sw.at[8]),
                2: pltpu.make_async_copy(wqkv_hbm.at[:, pl.ds(2 * D, D)], wraw.at[2], sw.at[9]),
                3: pltpu.make_async_copy(wo_hbm, wraw.at[3], sw.at[10])}

        def cp_f(c, s):
            o = _ds(c * FC, FC, FC)
            return [pltpu.make_async_copy(wg_hbm.at[:, o], raw[s][0], sf.at[3 * s]),
                    pltpu.make_async_copy(wu_hbm.at[:, o], raw[s][1], sf.at[3 * s + 1]),
                    pltpu.make_async_copy(wd_hbm.at[o, :], raw[s][2], sf.at[3 * s + 2])]

        def cp_o(t):
            return pltpu.make_async_copy(xb.at[_ds(t * TM, TM, TM)], o_hbm.at[_ds(t * TM, TM, TM)], so.at[t])

        def ln(src, dst, init=None):
            st = {}
            def mean(r):
                for i in range(2):
                    st[r, i] = jnp.sum(_sum([src(i * H + r, c) for c in range(NCB)]), axis=-1, keepdims=True) * (1.0 / D)
            def rstd(r):
                for i in range(2):
                    xc = [src(i * H + r, c) - st[r, i] for c in range(NCB)]
                    v = jnp.sum(_sum([a * a for a in xc]), axis=-1, keepdims=True) * (1.0 / D)
                    st[r, i, 1] = lax.rsqrt(v + 1e-5)
            def norm(r, c):
                h = [src(i * H + r, cc) for i in range(2) for cc in (c, c + 4)]
                a = [(h[n] - st[r, n // 2]) * st[r, n // 2, 1] for n in range(4)]
                for j, v in enumerate(_lhs7(*a)):
                    _put(dst, j, r, _cols(c), v)
                if init is not None:
                    z = jnp.zeros_like(h[0])
                    for j, v in enumerate((z, h[2], h[1], z, z, h[3] + h[2] - h[1], h[0])):
                        acc[j][init, r:r + 16, _cols(c)] = v
            def rows(lo=0, hi=H):
                out = []
                for r in range(lo, hi + 32, 16):
                    out += [P(mean, r)] if r < hi else []
                    out += [P(rstd, r - 16)] if lo + 16 <= r < hi + 16 else []
                    out += [P(norm, r - 32, c) for c in range(4)] if r >= lo + 32 else []
                return out
            return rows
        ln1 = lambda t: ln(lambda r, c: xb[pl.ds(t * TM + r, 16), _cols(c)].astype(F32), xa[t])
        ln2 = lambda t: ln(lambda r, c: hs[t][c, pl.ds(r, 16), :], ha.at[t], t)

        def prep_cols(m, t):
            st = {}
            def a(c):
                w = jnp.concatenate([wraw[m, _ds(b + t * 128, 128, 128), _cols(c)] for b in (0, DHALF)], axis=0)
                wt = pltpu.bitcast(w, U32).T
                for h in range(4):
                    tmp0[pl.ds((4 * c + h) * PITCH, DH), :] = wt[h * DH:(h + 1) * DH]
            def b(c):
                tmp1[_cols(c), :] = jnp.concatenate([tmp0[pl.ds(4 * c + d, NH, stride=PITCH), :] for d in range(4)], axis=0).T
            def e(c, r):
                g = lambda cc, rr: _bf(tmp1[pl.ds(cc * 128 + rr, 8), :])
                for j, v in enumerate(_rhs7(g(c, r), g(c + 4, r), g(c, r + 64), g(c + 4, r + 64))):
                    _put(wp[m], j, t * 128 + 2 * r, _cols(c), v)
            def e4(c, r):
                for rr in range(r, r + 32, 8):
                    e(c, rr)
            return ([P(a, c) for c in range(8)] + [P(b, c) for c in (0, 4, 1, 5, 2, 6, 3, 7)]
                    + [P(e4, c, r) for c in range(4) for r in (0, 32)])

        def prep_rows(t):
            def a(tmp, c, h0):
                for h in range(h0, h0 + 8):
                    tmp[pl.ds(h * PITCH, DH), :] = pltpu.bitcast(wraw[3, pl.ds(h * DH, DH), _ds(c * 128, 128, 128)].astype(F32), U32)
            def b(d):
                for h in (0, 16):
                    g = lambda tmp, dd: pltpu.bitcast(tmp[pl.ds(h * PITCH + dd, 16, stride=PITCH), :], F32)
                    for j, v in enumerate(_rhs7(g(tmp0, d), g(tmp1, d), g(tmp0, d + 16), g(tmp1, d + 16))):
                        _put(wp3, j, d * 32 + h, _cols(t), v)
            return [P(a, tm, c, h) for tm, c in ((tmp0, t), (tmp1, t + 4)) for h in range(0, NH, 8)] + [P(b, d) for d in range(16)]

        def prep_ffn(s, t):
            def piece(src, dst, kh, nh, r, c, oc):
                r = t * (kh // NT) + r
                g = lambda rr, cc: src[_ds(r + rr, 16, 16), pl.ds(c * 128 + cc, 128)]
                for j, v in enumerate(_rhs7(g(0, 0), g(0, nh), g(kh, 0), g(kh, nh))):
                    _put(dst, j, r, _cols(oc), v)
            g = GN // 128
            return ([P(piece, raw[s][i], fw[s][0], DHALF, FH, r, c, (c // g * 2 + i) * g + c % g)
                     for i in range(2) for r in range(0, DHALF // NT, 16) for c in range(FH // 128)]
                    + [P(piece, raw[s][2], fw[s][1], FH, DHALF, r, c, c) for r in range(0, FH // NT, 16) for c in range(4)])

        def probs(t):
            st = {}
            def a(r, w):
                ks = [kb[c, pl.ds(t * TM + r + HALO - DIL * w, 8), :] for c in range(NCB)]
                for rr, ww in ((r, w), (r + 8, w + 4)):
                    if 0 <= rr < TM:
                        st[rr, ww] = _sum([qb[c, pl.ds(t * TM + rr, 8), :] * ks[c] for c in range(NCB)])
            def b(r):
                l = jnp.concatenate([st[r, w] for w in range(WIN)], axis=0)
                st[r] = l + pltpu.roll(l, 64, 1)
            def e(r):
                l = st[r]
                l = (l + pltpu.roll(l, 32, 1)) * (DH ** -0.5 * LOG2E)
                ls = [l[w * 8:(w + 1) * 8] for w in range(WIN)]
                for w in range(WIN):
                    if t * TM + r < DIL * w:
                        pos = t * TM + r + lax.broadcasted_iota(jnp.int32, (8, 128), 0)
                        ls[w] = jnp.where(pos >= DIL * w, ls[w], -1e9 * LOG2E)
                m = functools.reduce(jnp.maximum, ls)
                ps = [jnp.exp2(l - m) for l in ls]
                inv = 1.0 / _sum(ps)
                for w in range(WIN):
                    pb[w, pl.ds(t * TM + r, 8), :] = ps[w] * inv
            def rows(lo, hi):
                out = [P(a2, lo - 8, w, lo, hi) for w in range(4)]
                for r in range(lo, hi, 8):
                    out += [P(a2, r, w, lo, hi) for w in range(4)] + [P(b, r)] + ([P(e, r - 8)] if r > lo else [])
                return out + [P(e, hi - 8)]
            def a2(r, w, lo, hi):
                ks = [kb[c, pl.ds(t * TM + r + HALO - DIL * w, 8), :] for c in range(NCB)]
                for rr, ww in ((r, w), (r + 8, w + 4)):
                    if lo <= rr < hi:
                        st[rr, ww] = _sum([qb[c, pl.ds(t * TM + rr, 8), :] * ks[c] for c in range(NCB)])
            return rows

        def pv(t):
            st = {}
            def part(r, c, i):
                r0 = t * TM + i * H + r
                for w in range(WIN):
                    p = pb[w, pl.ds(r0, 16), :]
                    a, b = (p * vb[cc, pl.ds(r0 + HALO - DIL * w, 16), :] for cc in (c, c + 4))
                    st[i] = (a, b) if w == 0 else (st[i][0] + a, st[i][1] + b)
                if i:
                    for j, v in enumerate(_lhs7(*st[0], *st[1])):
                        _put(xa[t], j, r, _cols(c), v)
            return lambda lo, hi: [P(part, r, c, i) for r in range(lo, hi, 16) for c in range(4) for i in range(2)]

        def zero_acc(t):
            def z(j, c):
                acc[j][t, :, _cols(c)] = jnp.zeros((H, 128), F32)
            return [P(z, j, c) for j in range(7) for c in range(4)]

        def proj(m, t, dst, off, resid, PM, lo=0, hi=H):
            for n in range(DHALF // PN):
                def emit(r, i, j, val):
                    for c in range(PN // 128):
                        cc = 4 * j + n * (PN // 128) + c
                        v = val[:, _cols(c)]
                        if resid:
                            v = v + xb[pl.ds(t * TM + i * H + r, PM), _cols(cc)].astype(F32)
                        dst[cc, pl.ds(off + i * H + r, PM), :] = v
                w = {}
                def prod(r, j):
                    if j not in w or not share:
                        w[j] = _bf(wp[m][j, :, _cols(n, PN)])
                    return _dot(_bf(xa[t][j, pl.ds(r // 2, PM // 2), :]), w[j])
                gens = [_strassen(P(prod, r), P(emit, r)) for r in range(lo, hi, PM)]
                if share:
                    for _ in range(7):
                        for g in gens:
                            next(g); yield
                else:
                    for g in gens:
                        yield from g

        cp_x0 = [[pltpu.make_async_copy(x_hbm.at[pl.ds(r, H // 2)], xb.at[pl.ds(r, H // 2)], s0.at[2 * i + j])
                  for j, r in enumerate((i * H // 2, H + i * H // 2))] for i in range(2)]
        units = [(cp_x0[0], ln1(0)(0, H // 2))] + [(cp_q[t], prep_cols(0, t)) for t in range(4)]
        queue = [u[0] for u in units] + [cp_x0[1], [cp_x[1]]]
        go[0] = 1
        for u in queue[:2]:
            for c in u:
                c.start()
        kb[:, 0:HALO, :] = jnp.zeros((NCB, HALO, 128), F32)
        for i, (cps, work) in enumerate(units):
            with scope(f'w{i}'):
                for c in cps:
                    c.wait()
            for c in queue[i + 2]:
                c.start()
            for f in work:
                f()
        with scope('wx1'):
            for c in cp_x0[1]:
                c.wait()
        cp_w[1].start()
        with scope('step0a'):
            _weave(proj(0, 0, qb, 0, False, H // 2, 0, H // 2), 7 * DHALF // PN, ln1(0)(H // 2, H), lead=lead)

        def keep():
            if only is not None:
                for a, b in ((xa0, xa1), (xa2, xa3), (wp0, wp1), (wp2, wp3), (kb, vb), (qb, pb)):
                    pltpu.sync_copy(a, b); pltpu.sync_copy(b, a)
        keep()

        ORDER = ((0, 0), (0, 1), (1, 0), (1, 1), (0, 2), (1, 2), (0, 3), (1, 3)) + tuple((m, t) for m in (2, 3) for t in range(NT))

        def span(fn, rows, unit, cuts, k):
            lo, hi = (int(round(cuts.get(i, 0 if i < min(cuts) else NT) * rows / unit)) * unit for i in (k - 1, k))
            out = []
            for t in range(NT):
                a, b = max(lo, t * rows) - t * rows, min(hi, (t + 1) * rows) - t * rows
                if a < b:
                    out += fn(t)(a, b)
            return out

        def step(k):
            m, t = ORDER[k]
            pm = PM.get(k, 256)
            lo = 0
            if k == 0:
                lo = pm = H // 2
                cp_x[1].wait()
                for c in [cp_x[2], cp_x[3], cp_w[2]]:
                    c.start()
            if k == 1:
                cp_w[1].wait()
            if k == 2:
                cp_x[2].wait(); cp_x[3].wait()
                for c in [cp_w[3]] + cp_f(0, 0) + cp_f(1, 1):
                    c.start()
            if k == 4:
                cp_w[2].wait()
            if k == 8:
                for c in [cp_w[3]] + cp_f(0, 0):
                    c.wait()
            if k == 9:
                for c in range(NCB):
                    vb[c, 0:HALO, :] = jnp.broadcast_to(vb[c, HALO:HALO + 1, :], (HALO, 128))
            sides = [span(ln1, H, 16, L1C, k), span(probs, TM, 8, PRC, k), span(pv, H, 16, PVC, k)]
            if k == 1:
                sides += [sum((prep_cols(1, i) for i in range(4)), [])]
            if k >= 4:
                sides += [(P(prep_cols, 2), prep_rows, P(prep_ffn, 0))[k // 4 - 1](k % 4)]
            sides += [span(ln2, H, 16, L2C, k)]
            if k < upto: _weave(proj(m, t, (qb, kb, vb, hs[t])[m], (t * TM, t * TM + HALO, t * TM + HALO, 0)[m], m == 3, pm, lo),
                   7 * DHALF // PN * ((H - lo) // pm), *sides, lead=lead * H // pm)

        k = 0
        while k < 4 * NT:
            ks = [k, k + 1] if k in merge else [k]
            with scope(f'step{k:02d}'):
                pl.when(go[0] > 0)(lambda: [step(i) for i in ks] and None)
            k += len(ks)

        def ffn(s, t, last):
            a = {}
            for n in range(FH // GN):
                def emit(i, j, val):
                    rows = []
                    for r in range(0, H, 16):
                        g, u = val[r:r + 16, :GN], val[r:r + 16, GN:]
                        rows.append((g * u) * (jnp.tanh(g * (g * g * C1 + C0)) * 0.5 + 0.5))
                    a[i, j, n] = jnp.concatenate(rows, axis=0)
                yield from _strassen(lambda j: _dot(_bf(ha[t, j]), _bf(fw[s][0][j, :, _cols(n, 2 * GN)])), emit)
            l7 = _lhs7(*(jnp.concatenate([a[i, j, n] for n in range(FH // GN)], axis=1) for i in range(2) for j in range(2)))
            l7 = [l.astype(BF16) for l in l7]
            dn = lambda j, n: acc[j][t, :, _cols(n, DN)] + _dot(l7[j], _bf(fw[s][1][j, :, _cols(n, DN)]))
            if not last:
                for j in (3, 1, 6, 2, 4, 0, 5):
                    for n in range(DHALF // DN):
                        acc[j][t, :, _cols(n, DN)] = dn(j, n)
                        yield
            else:
                for n in range(DHALF // DN):
                    def out(i, j, val):
                        for c in range(DN // 128):
                            cc = 4 * j + n * (DN // 128) + c
                            xb[_ds(t * TM + i * H, H, H), _cols(cc)] = val[:, _cols(c)].astype(BF16)
                        blk = (_ds(t * TM + i * H, H, H), pl.ds(j * DHALF + n * DN, DN))
                        pltpu.make_async_copy(xb.at[blk], o_hbm.at[blk], so).start()
                    m4 = dn(3, n); yield
                    m2 = dn(1, n); out(1, 0, m2 + m4); yield
                    c11 = m4 + dn(6, n); yield
                    m3 = dn(2, n); c22 = m3 - m2; yield
                    m5 = dn(4, n); out(0, 1, m3 + m5); c11 = c11 - m5; yield
                    m1 = dn(0, n); out(0, 0, c11 + m1); c22 = c22 + m1; yield
                    out(1, 1, c22 + dn(5, n)); yield
        NFF = 7 * (FH // GN + DHALF // DN)

        def body(s, t):
            _weave(ffn(s, t, False), NFF, prep_ffn(1 - s, t), lead=lead)

        def chunk(s, first):
            def it(i, _):
                for u in range(unroll):
                    body(s, i * unroll + u)
            lax.fori_loop(first, NT // unroll, it, None)

        def peeled():
            for c in cp_f(0, 1):
                c.wait()
            _weave(ffn(0, 0, False), NFF, prep_ffn(1, 0), span(ln2, H, 16, L2C, 16), lead=lead)
            for u in range(1, unroll):
                body(0, u)
        with scope('peel'):
            pl.when(go[0] > 0)(peeled)

        def pair(p, _):
            for c in cp_f(2 * p + 2, 0):
                c.start()
            @pl.when(p > 0)
            def _():
                for c in cp_f(0, 1):
                    c.wait()
            chunk(0, jnp.where(p == 0, 1, 0))
            @pl.when(p < NF // 2 - 1)
            def _():
                for c in cp_f(2 * p + 3, 1):
                    c.start()
            for c in cp_f(0, 0):
                c.wait()
            chunk(1, 0)
        if 'ffn' not in skip:
            with scope('ffn'):
                lax.fori_loop(0, NF // 2, pair, None)

        with scope('fin'):
            lax.fori_loop(0, NT, lambda t, _: _weave(ffn(0, t, True), NFF), None)
        pltpu.make_async_copy(xb, o_hbm, so).wait()

    def fn(A_x, A_wqkv, A_wo, B_x, B_w_gate, B_w_up, B_w_down):
        any_spec = pl.BlockSpec(memory_space=pl.ANY)
        V = pltpu.VMEM; DMA = pltpu.SemaphoreType.DMA
        out = pl.pallas_call(
            kernel, in_specs=[any_spec] * 6, out_specs=any_spec,
            out_shape=jax.ShapeDtypeStruct((S, D), BF16),
            scratch_shapes=[V((S, D), BF16), V((4, D, D), BF16)] + [V((7, D // 4, D // 2), U32)] * 4
                + [V((NH * PITCH, 128), U32)] * 2 + [V((7, H // 2, D // 2), U32)] * 4 + [V((NT, 7, H // 2, D // 2), U32)]
                + [V((NCB, S, 128), F32)] * 2 + [V((NCB, HALO + S, 128), F32)] * 2
                + [V((D, FC), BF16), V((D, FC), BF16), V((FC, D), BF16)] * 2
                + [V((7, D // 4, FC), U32), V((7, FH // 2, D // 2), U32)] * 2
                + [DMA((NT,)), DMA((11,)), DMA((6,)), DMA(()), DMA((4,)), pltpu.SMEM((1,), jnp.int32)]
                + [V((NT, H, D // 2), F32)] * 7,
            compiler_params=pltpu.CompilerParams(vmem_limit_bytes=vmem * 2 ** 20, flags=flags),
        )(A_x.reshape(S, D), A_wqkv, A_wo, B_w_gate, B_w_up, B_w_down)
        return out.reshape(1, S, D)
    return fn


_impl = make()


@jax.jit
def pallas_sequential_preLN__sliding_local_dilated__glu_gated_geglu__prompt_kernel(
    A_x, A_wqkv, A_wo, B_x, B_w_gate, B_w_up, B_w_down
):
    return _impl(A_x, A_wqkv, A_wo, B_x, B_w_gate, B_w_up, B_w_down)
```

```python
import contextlib
import functools

import jax
import jax.experimental.pallas as pl
import jax.experimental.pallas.tpu as pltpu
import jax.numpy as jnp
import numpy as np
from jax import lax

S, D, F = 2048, 1024, 3584
NH, DH, WIN, DIL = 32, 32, 8, 2
TM, FC = 512, 512
NT, NF = S // TM, F // FC
H, Q = TM // 2, TM // 4
NCB = D // 128
HALO = 16
PITCH = DH + 1
F32, BF16, U32 = jnp.float32, jnp.bfloat16, jnp.uint32
LOG2E = float(np.log2(np.e))
G0 = float(np.sqrt(2.0 / np.pi))
G1 = G0 * 0.044715
P = functools.partial

LHS = (((0, 1), (3, 1)), ((2, 1), (3, 1)), ((0, 1),), ((3, 1),), ((0, 1), (1, 1)), ((2, 1), (0, -1)), ((1, 1), (3, -1)))
RHS = (((0, 1), (3, 1)), ((0, 1),), ((1, 1), (3, -1)), ((2, 1), (0, -1)), ((3, 1),), ((0, 1), (1, 1)), ((2, 1), (3, 1)))
OUT = (((0, 1), (3, 1), (4, -1), (6, 1)), ((2, 1), (4, 1)), ((1, 1), (3, 1)), ((0, 1), (1, -1), (2, 1), (5, 1)))


def _comb(terms, get):
    v = get(terms[0][0])
    for i, sign in terms[1:]:
        a, b = v.astype(F32), get(i).astype(F32)
        v = a + b if sign > 0 else a - b
    return v


def _collector(emit):
    m = {}

    def push(j, val):
        m[j] = val
        for q, terms in enumerate(OUT):
            if j in dict(terms) and all(i in m for i, _ in terms):
                emit(q, _comb(terms, m.get))
    return push


def _block(q1, q2):
    return 2 * (q1 // 2) + q2 // 2, 2 * (q1 % 2) + q2 % 2


def _cols(c, n=128):
    return pl.ds(c * n, n)


def _ds(start, n, align):
    return pl.ds(start if isinstance(start, int) else pl.multiple_of(start, align), n)


def _bf(v):
    return pltpu.bitcast(v, BF16)


def _dot(a, b):
    return jnp.dot(_bf(a), _bf(b), preferred_element_type=F32)


def _put7(table, quads, dst, base, pair, col):
    for j, terms in enumerate(table):
        v = _comb(terms, quads.__getitem__).astype(BF16)
        dst.at[base + j][_ds(pair, 8, 8), _cols(col)] = pltpu.bitcast(v, U32)


def _weave(main, n, sides, lead=1):
    done = [0] * len(sides)
    for k in range(n):
        next(main)
        for s, side in enumerate(sides):
            upto = min(len(side), -(-len(side) * (k + 1) // (n - lead)))
            for job in side[done[s]:upto]:
                job()
            done[s] = upto


def _start(copies):
    for c in copies:
        c.start()


def _wait(copies):
    for c in copies:
        c.wait()


def make(PM={8: 128, 9: 128, 10: 128, 11: 64, 12: 64, 13: 128, 14: 128},
         L1C={-1: 1, 0: 2, 1: 2, 2: 3.25, 3: 3.5, 4: 3.75, 5: 4},
         PRC={3: .55, 4: 1.05, 5: 1.55, 6: 2.15, 7: 2.75, 8: 3.4, 9: 3.7, 10: 4},
         PVC={9: .5, 10: 1.0, 11: 2.0, 12: 3.0, 13: 3.5, 14: 4},
         L2C={13: .5, 14: 1, 15: 2, 16: 4},
         ZC={k: (k - 1) * .4 for k in range(2, 12)},
         FPC={12: 1, 13: 2, 14: 3, 15: 4},
         unroll=1, ahead=2, ffn_lead=3, scopes=False, skip=(), upto=16,
         flags={'XLA_TPU_EVENLY_DISTRIBUTE_CRITICAL_NODES': True}):
    scope = jax.named_scope if scopes else (lambda n: contextlib.nullcontext())

    def kernel(x_hbm, wqkv_hbm, wo_hbm, wg_hbm, wu_hbm, wd_hbm, o_hbm,
               xb, wraw, wp0, wp1, wp2, tmp0, tmp1, xa0, xa1, xa2, xa3, qb, kb, vb, ha, ab, acc,
               rg0, ru0, rd0, gu0, dn0, rg1, ru1, rd1, gu1, dn1, sx, sw, sf, so, go):
        xa = (xa0, xa1, xa2, xa3)
        wp = (wp0, wp1, wp2, wp0)
        raw = ((rg0, ru0, rd0), (rg1, ru1, rd1))
        gu, dn = (gu0, gu1), (dn0, dn1)
        copy = pltpu.make_async_copy

        def cp_x0(i):
            return [copy(x_hbm.at[pl.ds(r, Q)], xb.at[pl.ds(r, Q)], sx.at[r // Q]) for r in (i * Q, H + i * Q)]

        def cp_x(t):
            return [copy(x_hbm.at[pl.ds(t * TM, TM)], xb.at[pl.ds(t * TM, TM)], sx.at[3 + t])]

        def cp_q(i):
            return [copy(wqkv_hbm.at[pl.ds(r, 128), pl.ds(0, D)], wraw.at[0, pl.ds(r, 128)], sw.at[r // 128])
                    for r in (i * 128, D // 2 + i * 128)]

        def cp_w(m):
            return [copy(wqkv_hbm.at[:, pl.ds(m * D, D)] if m < 3 else wo_hbm, wraw.at[m % 2], sw.at[7 + m])]

        def cp_f(c, s):
            o = _ds(c * FC, FC, FC)
            return [copy(src, dst, sf.at[3 * s + i])
                    for i, (src, dst) in enumerate(zip((wg_hbm.at[:, o], wu_hbm.at[:, o], wd_hbm.at[o]), raw[s]))]

        def layernorm(load, parts, finish, lo, hi):
            st = {}

            def mean(r):
                for p in parts:
                    st[r, p] = jnp.sum(load(p + r).sum(0), axis=-1, keepdims=True) * (1.0 / D)

            def rstd(r):
                for p in parts:
                    xc = load(p + r) - st[r, p]
                    st[r, p, 1] = lax.rsqrt(jnp.sum((xc * xc).sum(0), axis=-1, keepdims=True) * (1.0 / D) + 1e-5)

            jobs = []
            for r in range(lo, hi + 32, 16):
                jobs += [P(mean, r)] if r < hi else []
                jobs += [P(rstd, r - 16)] if lo + 16 <= r < hi + 16 else []
                if r >= lo + 32:
                    jobs += finish(r - 32, lambda r, p, c: (load(p + r, c) - st[r, p]) * st[r, p, 1])
            return jobs

        def ln1(t, lo, hi):
            def load(r, c=None):
                get = lambda c: xb[pl.ds(t * TM + r, 16), _cols(c)].astype(F32)
                return jnp.stack([get(c) for c in range(NCB)]) if c is None else get(c)

            def put(r, c, norm):
                _put7(LHS, [norm(r, q // 2 * H, q % 2 * 4 + c) for q in range(4)], xa[t], 0, r // 2, c)
            return layernorm(load, (0, H), lambda r, norm: [P(put, r, c, norm) for c in range(4)], lo, hi)

        def ln2(t, lo, hi):
            def load(r, c=slice(None)):
                return qb[c, pl.ds(t * TM + r, 16), :]

            def finish(r, norm):
                @functools.cache
                def get(c, q1, q2):
                    i, k = _block(q1, q2)
                    return norm(r, i * Q, 2 * k + c)

                def put(c, j):
                    _put7(LHS, [_comb(LHS[j], lambda q1: get(c, q1, q2)) for q2 in range(4)], ha.at[t], 7 * j, r // 2, c)
                return [P(put, c, j) for c in range(2) for j in range(7)]
            return layernorm(load, (0, Q, 2 * Q, 3 * Q), finish, lo, hi)

        def prep_cols(m, i):
            def fwd(c):
                w = jnp.concatenate([wraw[m % 2, pl.ds(b + i * 128, 128), _cols(c)] for b in (0, D // 2)], axis=0)
                wt = pltpu.bitcast(w, U32).T
                for h in range(4):
                    tmp0[pl.ds((4 * c + h) * PITCH, DH), :] = wt[h * DH:(h + 1) * DH]

            def back(c):
                rows = [tmp0[pl.ds(4 * c + d, NH, stride=PITCH), :] for d in range(4)]
                tmp1[_cols(c), :] = jnp.concatenate(rows, axis=0).T

            def put(c, r0):
                for r in range(r0, r0 + 32, 8):
                    quads = [_bf(tmp1[pl.ds((q % 2 * 4 + c) * 128 + q // 2 * 64 + r, 8), :]) for q in range(4)]
                    _put7(RHS, quads, wp[m], 0, i * 64 + r, c)
            return ([P(fwd, c) for c in range(NCB)] + [P(back, c) for c in (0, 4, 1, 5, 2, 6, 3, 7)]
                    + [P(put, c, r) for c in range(4) for r in (0, 32)])

        def prep_rows(i):
            def fwd(n, h0):
                for h in range(h0, h0 + 8):
                    w = wraw[1, pl.ds(h * DH, DH), _cols(4 * n + i)].astype(F32)
                    (tmp0, tmp1)[n][pl.ds(h * PITCH, DH), :] = pltpu.bitcast(w, U32)

            def put(d):
                for h in (0, 16):
                    quads = [(tmp0, tmp1)[q % 2][pl.ds(h * PITCH + q // 2 * 16 + d, 16, stride=PITCH), :] for q in range(4)]
                    _put7(RHS, [pltpu.bitcast(v, F32) for v in quads], wp[3], 0, d * 16 + h // 2, i)
            return [P(fwd, n, h) for n in range(2) for h in range(0, NH, 8)] + [P(put, d) for d in range(16)]

        def prep_ffn(s, t, lo=0, hi=84):
            def put(src, dst, kb_, nb, r, c, col, j):
                def get(q1, q2):
                    k, n = _block(q1, q2)
                    return src[_ds(k * kb_ + t * (kb_ // NT) + r, 16, 16), pl.ds(n * nb + c * 128, 128)]
                quads = [_comb(RHS[j], lambda q1: get(q1, q2)) for q2 in range(4)]
                _put7(RHS, quads, dst, 7 * j, t * (kb_ // NT // 2) + r // 2, col)
            jobs = [P(put, raw[s][i], gu[s], D // 4, FC // 4, r, 0, i, j)
                    for i in range(2) for r in range(0, D // 4 // NT, 16) for j in range(7)]
            jobs += [P(put, raw[s][2], dn[s], FC // 4, D // 4, r, c, c, j)
                     for c in range(2) for r in range(0, FC // 4 // NT, 16) for j in range(7)]
            return jobs[lo:hi]

        def probs(t, lo, hi):
            st = {}

            def dots(r, w):
                k = kb[:, pl.ds(t * TM + r + HALO - DIL * w, 8), :]
                for rr, ww in ((r, w), (r + 8, w + 8 // DIL)):
                    if lo <= rr < hi:
                        st[rr, ww] = (qb[:, pl.ds(t * TM + rr, 8), :] * k).sum(0)

            def fold(r):
                l = jnp.concatenate([st[r, w] for w in range(WIN)], axis=0)
                st[r] = l + pltpu.roll(l, 64, 1)

            def softmax(r):
                l = (st[r] + pltpu.roll(st[r], 32, 1)) * (DH ** -0.5 * LOG2E)
                l = l.reshape(WIN, 8, 128)
                if t * TM + r < DIL * (WIN - 1):
                    pos = t * TM + r + lax.broadcasted_iota(jnp.int32, l.shape, 1)
                    l = jnp.where(pos >= DIL * lax.broadcasted_iota(jnp.int32, l.shape, 0), l, -1e9 * LOG2E)
                p = jnp.exp2(l - l.max(0))
                qb[:, pl.ds(t * TM + r, 8), :] = p * (1.0 / p.sum(0))

            jobs = [P(dots, lo - 8, w) for w in range(4)]
            for r in range(lo, hi, 8):
                jobs += [P(dots, r, w) for w in range(4)] + [P(fold, r)] + ([P(softmax, r - 8)] if r > lo else [])
            return jobs + [P(softmax, hi - 8)]

        def mix(t, lo, hi):
            st = {}

            def part(r, c, i):
                r0 = t * TM + i * H + r
                for w in range(WIN):
                    pv = qb[w, pl.ds(r0, 16), :] * vb[pl.ds(2 * c, 2), pl.ds(r0 + HALO - DIL * w, 16), :]
                    st[i] = st[i] + pv if w else pv
                if i:
                    _put7(LHS, [st[q // 2][q % 2] for q in range(4)], xa[t], 0, r // 2, c)
            return [P(part, r, c, i) for r in range(lo, hi, 16) for c in range(4) for i in range(2)]

        def clear(t, lo, hi):
            def job(j):
                acc[t, j // 4, pl.ds(j % 4 * 32, 32), :] = jnp.zeros((32, D // 4), F32)
            return [P(job, j) for j in range(lo, hi)]

        def span(fn, size, unit, cuts, k):
            lo, hi = (int(round(cuts.get(i, 0 if i < min(cuts) else NT) * size / unit)) * unit for i in (k - 1, k))
            jobs = []
            for t in range(NT):
                a, b = max(lo - t * size, 0), min(hi - t * size, size)
                jobs += fn(t, a, b) if a < b else []
            return jobs

        def project(m, t, rows, lo, hi, sides):
            def stages():
                for n in range(4):
                    for r in range(lo, hi, rows):
                        def emit(q, val):
                            r0, c = t * TM + q // 2 * H + r, q % 2 * 4 + n
                            if m == 0:
                                qb[c, pl.ds(r0, rows), :] = val
                            elif m == 1:
                                kb[c, pl.ds(HALO + r0, rows), :] = val
                            elif m == 2:
                                vb[2 * n + q % 2, pl.ds(HALO + r0, rows), :] = val
                            else:
                                qb[c, pl.ds(r0, rows), :] = val + xb[pl.ds(r0, rows), _cols(c)].astype(F32)
                        push = _collector(emit)
                        for j in range(7):
                            push(j, _dot(xa[t][j, pl.ds(r // 2, rows // 2), :], wp[m][j, :, _cols(n)]))
                            yield
            n = (hi - lo) // rows
            _weave(stages(), 28 * n, sides, lead=n)

        units = [(cp_x0(0), ln1(0, 0, Q))] + [(cp_q(i), prep_cols(0, i)) for i in range(4)]
        queue = [u[0] for u in units] + [cp_x0(1), cp_x(1)]
        go[0] = 1
        _start(queue[0] + queue[1])
        kb[:, pl.ds(0, HALO), :] = jnp.zeros((NCB, HALO, 128), F32)
        for i, (copies, jobs) in enumerate(units):
            with scope(f'w{i}'):
                _wait(copies)
            _start(queue[i + 2])
            for job in jobs:
                job()
        _wait(cp_x0(1))
        _start(cp_w(1))
        with scope('step0a'):
            project(0, 0, Q, 0, Q, [ln1(0, Q, H)])

        order = ((0, 0), (0, 1), (1, 0), (1, 1), (0, 2), (1, 2), (0, 3), (1, 3)) + tuple((m, t) for m in (2, 3) for t in range(NT))

        def step(k):
            sides = []
            if k == 0:
                _wait(cp_x(1))
                _start(cp_x(2) + cp_x(3) + cp_w(2))
            elif k == 1:
                _wait(cp_w(1))
                sides.append(sum((prep_cols(1, i) for i in range(4)), []))
            elif k == 2:
                _wait(cp_x(2) + cp_x(3))
                _start(cp_w(3) + cp_f(0, 0) + cp_f(1, 1))
            elif k == 4:
                _wait(cp_w(2))
            elif k == 8:
                _wait(cp_w(3) + cp_f(0, 0))
            elif k == 9:
                vb[:, pl.ds(0, HALO), :] = jnp.broadcast_to(vb[:, pl.ds(HALO, 1), :], (NCB, HALO, 128))
            if 4 <= k < 12:
                sides.append(prep_cols(2, k - 4) if k < 8 else prep_rows(k - 8))
            sides = [span(ln1, H, 16, L1C, k), span(probs, TM, 8, PRC, k), span(mix, H, 16, PVC, k)] + sides + [
                span(P(prep_ffn, 0), 84, 1, FPC, k), span(ln2, Q, 16, L2C, k), span(clear, 196, 1, ZC, k)]
            if k < upto:
                project(*order[k], PM.get(k, H) if k else Q, 0 if k else Q, H, sides)

        for k in range(4 * NT):
            with scope(f'step{k:02d}'):
                pl.when(go[0] > 0)(P(step, k))

        def ffn(s, t, sides, last=False):
            act = {}

            def geglu(q2, q1, val):
                for r in range(0, Q, 16):
                    g, u = val[r:r + 16, :128], val[r:r + 16, 128:]
                    act[q1, q2, r] = (g * u) * (jnp.tanh(g * (g * g * G1 + G0)) * 0.5 + 0.5)

            def store(q2, q1, val):
                i, n = _block(q1, q2)
                rows = _ds(t * TM + i * Q, Q, Q)
                for c in range(2):
                    xb[rows, _cols(2 * n + c)] = (qb[2 * n + c, rows, :] + val[:, c * 128:(c + 1) * 128]).astype(BF16)
                copy(xb.at[rows, _cols(n, 256)], o_hbm.at[rows, _cols(n, 256)], so).start()

            def products(j1, outer, product):
                inner = _collector(lambda q2, v: outer[q2](j1, v))
                for j2 in range(7):
                    inner(j2, product(7 * j1 + j2))
                    yield

            def operands(j1):
                for r in range(0, Q, 16):
                    _put7(LHS, [_comb(LHS[j1], lambda q1: act[q1, q2, r]) for q2 in range(4)], ab, 7 * j1, r // 2, 0)

            def stages():
                up = [_collector(P(geglu, q2)) for q2 in range(4)]
                out = [_collector(P(store, q2)) for q2 in range(4)]
                down = lambda j: acc[t, j] + _dot(ab[j], dn[s][j])
                seq = (3, 1, 6, 2, 4, 0, 5)
                for j1 in range(7):
                    if j1 == 6:
                        for j in seq[:ahead]:
                            operands(j)
                    yield from products(j1, up, lambda j: _dot(ha[t, j], gu[s][j]))
                for n, j1 in enumerate(seq):
                    if last:
                        yield from products(j1, out, down)
                    else:
                        for j in range(7 * j1, 7 * j1 + 7):
                            acc[t, j] = down(j)
                            yield
                    if n + ahead < 7:
                        operands(seq[n + ahead])
            _weave(stages(), 98, sides, lead=ffn_lead)

        def chunk(s, first):
            def body(i, _):
                for u in range(unroll):
                    ffn(s, i * unroll + u, [prep_ffn(1 - s, i * unroll + u)])
            lax.fori_loop(first, NT // unroll, body, None)

        def peeled(u):
            if u == 0:
                _wait(cp_f(1, 1))
            ffn(0, u, [prep_ffn(1, u), span(ln2, Q, 16, L2C, 16 + u)])
        for u in range(unroll):
            with scope('peel'):
                pl.when(go[0] > 0)(P(peeled, u))

        def pair(p, _):
            _start(cp_f(2 * p + 2, 0))
            pl.when(p > 0)(lambda: _wait(cp_f(2 * p + 1, 1)))
            chunk(0, jnp.where(p == 0, 1, 0))
            pl.when(p < NF // 2 - 1)(lambda: _start(cp_f(2 * p + 3, 1)))
            _wait(cp_f(2 * p + 2, 0))
            chunk(1, 0)
        if 'ffn' not in skip:
            with scope('ffn'):
                lax.fori_loop(0, NF // 2, pair, None)
        with scope('fin'):
            lax.fori_loop(0, NT, lambda t, _: ffn(0, t, [], last=True), None)
        copy(xb, o_hbm, so).wait()

    def fn(A_x, A_wqkv, A_wo, B_x, B_w_gate, B_w_up, B_w_down):
        hbm = pl.BlockSpec(memory_space=pl.ANY)
        V, DMA = pltpu.VMEM, pltpu.SemaphoreType.DMA
        out = pl.pallas_call(
            kernel, in_specs=[hbm] * 6, out_specs=hbm,
            out_shape=jax.ShapeDtypeStruct((S, D), BF16),
            scratch_shapes=(
                [V((S, D), BF16), V((2, D, D), BF16)] + [V((7, D // 4, D // 2), U32)] * 3
                + [V((NH * PITCH, 128), U32)] * 2 + [V((7, H // 2, D // 2), U32)] * NT
                + [V((NCB, S, 128), F32)] + [V((NCB, HALO + S, 128), F32)] * 2
                + [V((NT, 49, Q // 2, D // 4), U32), V((49, Q // 2, FC // 4), U32), V((NT, 49, Q, D // 4), F32)]
                + [V((D, FC), BF16), V((D, FC), BF16), V((FC, D), BF16),
                   V((49, D // 8, FC // 2), U32), V((49, FC // 8, D // 4), U32)] * 2
                + [DMA((7,)), DMA((11,)), DMA((6,)), DMA(()), pltpu.SMEM((1,), jnp.int32)]),
            compiler_params=pltpu.CompilerParams(vmem_limit_bytes=122 * 2 ** 20, flags=flags),
        )(A_x.reshape(S, D), A_wqkv, A_wo, B_w_gate, B_w_up, B_w_down)
        return out.reshape(1, S, D)
    return fn


_impl = make()


@jax.jit
def pallas_sequential_preLN__sliding_local_dilated__glu_gated_geglu__prompt_kernel(
    A_x, A_wqkv, A_wo, B_x, B_w_gate, B_w_up, B_w_down
):
    return _impl(A_x, A_wqkv, A_wo, B_x, B_w_gate, B_w_up, B_w_down)
```

```python
import contextlib
import functools

import jax
import jax.experimental.pallas as pl
import jax.experimental.pallas.tpu as pltpu
import jax.numpy as jnp
import numpy as np
from jax import lax

S, D, F = 2048, 1024, 3584
NH, DH, WIN, DIL = 32, 32, 8, 2
TM, FC = 512, 512
NT, NF = S // TM, F // FC
H, Q = TM // 2, TM // 4
NCB = D // 128
HALO = 16
PITCH = DH + 1
F32, BF16, U32 = jnp.float32, jnp.bfloat16, jnp.uint32
LOG2E = float(np.log2(np.e))
G0 = float(np.sqrt(2.0 / np.pi))
G1 = G0 * 0.044715
P = functools.partial

LHS = (((0, 1), (3, 1)), ((2, 1), (3, 1)), ((0, 1),), ((3, 1),), ((0, 1), (1, 1)), ((2, 1), (0, -1)), ((1, 1), (3, -1)))
RHS = (((0, 1), (3, 1)), ((0, 1),), ((1, 1), (3, -1)), ((2, 1), (0, -1)), ((3, 1),), ((0, 1), (1, 1)), ((2, 1), (3, 1)))
OUT = (((0, 1), (3, 1), (4, -1), (6, 1)), ((2, 1), (4, 1)), ((1, 1), (3, 1)), ((0, 1), (1, -1), (2, 1), (5, 1)))


def _comb(terms, get):
    v = get(terms[0][0])
    for i, sign in terms[1:]:
        a, b = v.astype(F32), get(i).astype(F32)
        v = a + b if sign > 0 else a - b
    return v


def _collector(emit):
    part = {}

    def push(j, val):
        for q, terms in enumerate(OUT):
            sign = dict(terms).get(j)
            if sign is None:
                continue
            if q not in part:
                part[q] = (val, sign, 1)
                continue
            v, s, n = part[q]
            v = v + val if s == sign else v - val if s > 0 else val - v
            part[q] = (v, 1, n + 1)
            if n + 1 == len(terms):
                emit(q, v)
    return push


def _block(q1, q2):
    return 2 * (q1 // 2) + q2 // 2, 2 * (q1 % 2) + q2 % 2


def _cols(c, n=128):
    return pl.ds(c * n, n)


def _ds(start, n, align):
    return pl.ds(start if isinstance(start, int) else pl.multiple_of(start, align), n)


def _bf(v):
    return pltpu.bitcast(v, BF16)


def _dot(a, b):
    return jnp.dot(_bf(a), _bf(b), preferred_element_type=F32)


def _put7(table, quads, dst, base, pair, col):
    for j, terms in enumerate(table):
        v = _comb(terms, quads.__getitem__).astype(BF16)
        dst.at[base + j][_ds(pair, 8, 8), _cols(col)] = pltpu.bitcast(v, U32)


def _weave(main, n, sides, lead=1):
    done = [0] * len(sides)
    for k in range(n):
        next(main)
        for s, side in enumerate(sides):
            upto = min(len(side), -(-len(side) * (k + 1) // (n - lead)))
            for job in side[done[s]:upto]:
                job()
            done[s] = upto


def _start(copies):
    for c in copies:
        c.start()


def _wait(copies):
    for c in copies:
        c.wait()


def make(PM={9: 128, 10: 64, 11: 64, 12: 64},
         L1C={-1: 1, 0: 2, 1: 2.5, 2: 3.75, 3: 4},
         PRC={3: .55, 4: 1.15, 5: 1.75, 6: 2.4, 7: 3, 8: 3.65, 9: 4},
         PVC={9: .625, 10: 1.75, 11: 2.875, 12: 4},
         L2C={13: 1, 14: 2, 15: 3, 16: 4},
         FPC={3: .5, 4: 1, 5: 1.5, 6: 1.75, 7: 2.25, 8: 2.5, 9: 2.5, 10: 2.75, 11: 3, 12: 3.5, 13: 3.75, 14: 4}, F1K=15,
         unroll=1, ahead=3, ffn_lead=3, first_lead=3, peel=1, PROJ=(1, 3, 6, 4, 2, 0, 5), INNER=(1, 3, 6, 4, 2, 0, 5), plan='0 4 6 3 1//2 2//5 5//4 /2/3 /5/1 /4/6 /3/0 /1 /6 /0', last='0 1 2 5 3//3 4//1 6//6 /3/2 /1/4 /6/0 /2/5 /4 /0 /5', cache=True, LP=2, scopes=False, skip=(), upto=16,
         flags={'XLA_TPU_EVENLY_DISTRIBUTE_CRITICAL_NODES': True}):
    PLAN, PLAN_LAST = ([[[int(c) for c in f] for f in (w + '//').split('/')[:3]] for w in p.split()] for p in (plan, last))
    scope = jax.named_scope if scopes else (lambda n: contextlib.nullcontext())

    def kernel(x_hbm, wqkv_hbm, wo_hbm, wg_hbm, wu_hbm, wd_hbm, o_hbm,
               xb, wraw, wp0, wp1, wp2, tmp0, tmp1, xa0, xa1, xa2, xa3, qb, kb, vb, ha, ab, acc,
               rg0, ru0, rd0, gu0, dn0, rg1, ru1, rd1, gu1, dn1, sx, sw, sf, so, go):
        xa = (xa0, xa1, xa2, xa3)
        wp = (wp0, wp1, wp2, wp0)
        raw = ((rg0, ru0, rd0), (rg1, ru1, rd1))
        gu, dn = (gu0, gu1), (dn0, dn1)
        copy = pltpu.make_async_copy

        def cp_x0(i):
            return [copy(x_hbm.at[pl.ds(r, Q)], xb.at[pl.ds(r, Q)], sx.at[r // Q]) for r in (i * Q, H + i * Q)]

        def cp_x(t):
            return [copy(x_hbm.at[pl.ds(t * TM, TM)], xb.at[pl.ds(t * TM, TM)], sx.at[3 + t])]

        def cp_q(i):
            return [copy(wqkv_hbm.at[pl.ds(r, 128), pl.ds(0, D)], wraw.at[0, pl.ds(r, 128)], sw.at[r // 128])
                    for r in (i * 128, D // 2 + i * 128)]

        def cp_w(m):
            return [copy(wqkv_hbm.at[:, pl.ds(m * D, D)] if m < 3 else wo_hbm, wraw.at[m % 2], sw.at[7 + m])]

        def cp_f(c, s):
            o = _ds(c * FC, FC, FC)
            return [copy(src, dst, sf.at[3 * s + i])
                    for i, (src, dst) in enumerate(zip((wg_hbm.at[:, o], wu_hbm.at[:, o], wd_hbm.at[o]), raw[s]))]

        def layernorm(load, parts, finish, lo, hi):
            st = {}

            def mean(r, *parts):
                for p in parts:
                    st[r, p] = jnp.sum(load(p + r).sum(0), axis=-1, keepdims=True) * (1.0 / D)

            def rstd(r, *parts):
                for p in parts:
                    xc = load(p + r) - st[r, p]
                    st[r, p, 1] = lax.rsqrt(jnp.sum((xc * xc).sum(0), axis=-1, keepdims=True) * (1.0 / D) + 1e-5)

            jobs = []
            for r in range(lo, hi + 32, 16):
                jobs += [P(mean, r, *parts[i:i + LP]) for i in range(0, len(parts), LP)] if r < hi else []
                jobs += [P(rstd, r - 16, *parts[i:i + LP]) for i in range(0, len(parts), LP)] if lo + 16 <= r < hi + 16 else []
                if r >= lo + 32:
                    jobs += finish(r - 32, lambda r, p, c: (load(p + r, c) - st[r, p]) * st[r, p, 1])
            return jobs

        def ln1(t, lo, hi):
            def load(r, c=None):
                get = lambda c: xb[pl.ds(t * TM + r, 16), _cols(c)].astype(F32)
                return jnp.stack([get(c) for c in range(NCB)]) if c is None else get(c)

            def put(r, c, norm):
                _put7(LHS, [norm(r, q // 2 * H, q % 2 * 4 + c) for q in range(4)], xa[t], 0, r // 2, c)
            return layernorm(load, (0, H), lambda r, norm: [P(put, r, c, norm) for c in range(4)], lo, hi)

        def ln2(t, lo, hi):
            def load(r, c=slice(None)):
                return qb[c, pl.ds(t * TM + r, 16), :]

            def finish(r, norm):
                @(functools.cache if cache else lambda f: f)
                def get(c, q1, q2):
                    i, k = _block(q1, q2)
                    return norm(r, i * Q, 2 * k + c)

                def put(c, j):
                    _put7(LHS, [_comb(LHS[j], lambda q1: get(c, q1, q2)) for q2 in range(4)], ha.at[t], 7 * j, r // 2, c)
                return [P(put, c, j) for c in range(2) for j in range(7)]
            return layernorm(load, (0, Q, 2 * Q, 3 * Q), finish, lo, hi)

        def prep_cols(m, i):
            def fwd(c):
                w = jnp.concatenate([wraw[m % 2, pl.ds(b + i * 128, 128), _cols(c)] for b in (0, D // 2)], axis=0)
                wt = pltpu.bitcast(w, U32).T
                for h in range(4):
                    tmp0[pl.ds((4 * c + h) * PITCH, DH), :] = wt[h * DH:(h + 1) * DH]

            def back(c):
                rows = [tmp0[pl.ds(4 * c + d, NH, stride=PITCH), :] for d in range(4)]
                tmp1[_cols(c), :] = jnp.concatenate(rows, axis=0).T

            def put(c, r0):
                for r in range(r0, r0 + 32, 8):
                    quads = [_bf(tmp1[pl.ds((q % 2 * 4 + c) * 128 + q // 2 * 64 + r, 8), :]) for q in range(4)]
                    _put7(RHS, quads, wp[m], 0, i * 64 + r, c)
            return ([P(fwd, c) for c in range(NCB)] + [P(back, c) for c in (0, 4, 1, 5, 2, 6, 3, 7)]
                    + [P(put, c, r) for c in range(4) for r in (0, 32)])

        def prep_rows(i):
            def fwd(n, h0):
                for h in range(h0, h0 + 2):
                    w = wraw[1, pl.ds(h * DH, DH), _cols(4 * n + i)].astype(F32)
                    (tmp0, tmp1)[n][pl.ds(h * PITCH, DH), :] = pltpu.bitcast(w, U32)

            def put(d):
                for h in (0, 16):
                    quads = [(tmp0, tmp1)[q % 2][pl.ds(h * PITCH + q // 2 * 16 + d, 16, stride=PITCH), :] for q in range(4)]
                    _put7(RHS, [pltpu.bitcast(v, F32) for v in quads], wp[3], 0, d * 16 + h // 2, i)
            return [P(fwd, n, h) for n in range(2) for h in range(0, NH, 2)] + [P(put, d) for d in range(16)]

        def prep_ffn(s, t, lo=0, hi=84):
            def put(src, dst, kb_, nb, r, c, col, j):
                def get(q1, q2):
                    k, n = _block(q1, q2)
                    return src[_ds(k * kb_ + t * (kb_ // NT) + r, 16, 16), pl.ds(n * nb + c * 128, 128)]
                quads = [_comb(RHS[j], lambda q1: get(q1, q2)) for q2 in range(4)]
                _put7(RHS, quads, dst, 7 * j, t * (kb_ // NT // 2) + r // 2, col)
            jobs = [P(put, raw[s][i], gu[s], D // 4, FC // 4, r, 0, i, j)
                    for i in range(2) for r in range(0, D // 4 // NT, 16) for j in range(7)]
            jobs += [P(put, raw[s][2], dn[s], FC // 4, D // 4, r, c, c, j)
                     for c in range(2) for r in range(0, FC // 4 // NT, 16) for j in range(7)]
            return jobs[lo:hi]

        def probs(t, lo, hi):
            st = {}

            def dots(r, w):
                k = kb[:, pl.ds(t * TM + r + HALO - DIL * w, 8), :]
                for rr, ww in ((r, w), (r + 8, w + 8 // DIL)):
                    if lo <= rr < hi:
                        st[rr, ww] = (qb[:, pl.ds(t * TM + rr, 8), :] * k).sum(0)

            def fold(r):
                l = jnp.concatenate([st[r, w] for w in range(WIN)], axis=0)
                st[r] = l + pltpu.roll(l, 64, 1)

            def softmax(r):
                l = (st[r] + pltpu.roll(st[r], 32, 1)) * (DH ** -0.5 * LOG2E)
                l = l.reshape(WIN, 8, 128)
                if t * TM + r < DIL * (WIN - 1):
                    pos = t * TM + r + lax.broadcasted_iota(jnp.int32, l.shape, 1)
                    l = jnp.where(pos >= DIL * lax.broadcasted_iota(jnp.int32, l.shape, 0), l, -1e9 * LOG2E)
                p = jnp.exp2(l - l.max(0))
                qb[:, pl.ds(t * TM + r, 8), :] = p * (1.0 / p.sum(0))

            jobs = [P(dots, lo - 8, w) for w in range(4)]
            for r in range(lo, hi, 8):
                jobs += [P(dots, r, w) for w in range(4)] + [P(fold, r)] + ([P(softmax, r - 8)] if r > lo else [])
            return jobs + [P(softmax, hi - 8)]

        def mix(t, lo, hi):
            st = {}

            def part(r, c, i):
                r0 = t * TM + i * H + r
                for w in range(WIN):
                    pv = qb[w, pl.ds(r0, 16), :] * vb[pl.ds(2 * c, 2), pl.ds(r0 + HALO - DIL * w, 16), :]
                    st[i] = st[i] + pv if w else pv
                if i:
                    _put7(LHS, [st[q // 2][q % 2] for q in range(4)], xa[t], 0, r // 2, c)
            return [P(part, r, c, i) for r in range(lo, hi, 16) for c in range(4) for i in range(2)]

        def span(fn, size, unit, cuts, k):
            lo, hi = (int(round(cuts.get(i, 0 if i < min(cuts) else NT) * size / unit)) * unit for i in (k - 1, k))
            jobs = []
            for t in range(NT):
                a, b = max(lo - t * size, 0), min(hi - t * size, size)
                jobs += fn(t, a, b) if a < b else []
            return jobs

        def project(m, t, rows, lo, hi, sides):
            def stages():
                for n in range(4):
                    for r in range(lo, hi, rows):
                        def emit(q, val):
                            r0, c = t * TM + q // 2 * H + r, q % 2 * 4 + n
                            if m == 0:
                                qb[c, pl.ds(r0, rows), :] = val
                            elif m == 1:
                                kb[c, pl.ds(HALO + r0, rows), :] = val
                            elif m == 2:
                                vb[2 * n + q % 2, pl.ds(HALO + r0, rows), :] = val
                            else:
                                qb[c, pl.ds(r0, rows), :] = val + xb[pl.ds(r0, rows), _cols(c)].astype(F32)
                        push = _collector(emit)
                        for j in PROJ:
                            push(j, _dot(xa[t][j, pl.ds(r // 2, rows // 2), :], wp[m][j, :, _cols(n)]))
                            yield
            n = (hi - lo) // rows
            _weave(stages(), 28 * n, sides, lead=n)

        units = [(cp_x0(0), ln1(0, 0, Q))] + [(cp_q(i), prep_cols(0, i)) for i in range(4)]
        queue = [u[0] for u in units] + [cp_x0(1), cp_x(1)]
        go[0] = 1
        _start(queue[0] + queue[1])
        kb[:, pl.ds(0, HALO), :] = jnp.zeros((NCB, HALO, 128), F32)
        for i, (copies, jobs) in enumerate(units):
            with scope(f'w{i}'):
                _wait(copies)
            _start(queue[i + 2])
            for job in jobs:
                job()
        _wait(cp_x0(1))
        _start(cp_w(1))
        with scope('step0a'):
            project(0, 0, Q, 0, Q, [ln1(0, Q, H)])

        order = ((0, 0), (0, 1), (1, 0), (1, 1), (0, 2), (1, 2), (0, 3), (1, 3)) + tuple((m, t) for m in (2, 3) for t in range(NT))

        def step(k):
            sides = []
            if k == 0:
                _wait(cp_x(1))
                _start(cp_x(2) + cp_x(3) + cp_f(0, 0) + cp_w(2))
            elif k == 1:
                _wait(cp_w(1) + cp_x(2))
                sides.append(sum((prep_cols(1, i) for i in range(4)), []))
            elif k == 2:
                _wait(cp_x(3))
                _start(cp_w(3) + cp_f(1, 1))
            elif k == 3:
                _wait(cp_f(0, 0))
            elif k == 4:
                _wait(cp_w(2))
            elif k == 8:
                _wait(cp_w(3) + cp_f(1, 1))
            elif k == 9:
                vb[:, pl.ds(0, HALO), :] = jnp.broadcast_to(vb[:, pl.ds(HALO, 1), :], (NCB, HALO, 128))
            if 4 <= k < 12:
                sides.append(prep_cols(2, k - 4) if k < 8 else prep_rows(k - 8))
            sides = [span(ln1, H, 16, L1C, k), span(probs, TM, 8, PRC, k), span(mix, H, 16, PVC, k)] + sides + [
                span(P(prep_ffn, 0), 84, 1, FPC, k), span(ln2, Q, 16, L2C, k)]
            if k == F1K:
                sides.append(prep_ffn(1, 0))
            if k < upto:
                project(*order[k], PM.get(k, H) if k else Q, 0 if k else Q, H, sides)

        for k in range(4 * NT):
            with scope(f'step{k:02d}'):
                pl.when(go[0] > 0)(P(step, k))

        def ffn(s, t, sides, first=False, last=False, lead=ffn_lead):
            act = {}

            def geglu(q2, q1, val):
                for r in range(0, Q, 16):
                    g, u = val[r:r + 16, :128], val[r:r + 16, 128:]
                    act[q1, q2, r] = (g * u) * (jnp.tanh(g * (g * g * G1 + G0)) * 0.5 + 0.5)

            def store(q2, q1, val):
                i, n = _block(q1, q2)
                rows = _ds(t * TM + i * Q, Q, Q)
                for c in range(2):
                    xb[rows, _cols(2 * n + c)] = (qb[2 * n + c, rows, :] + val[:, c * 128:(c + 1) * 128]).astype(BF16)
                copy(xb.at[rows, _cols(n, 256)], o_hbm.at[rows, _cols(n, 256)], so).start()

            def products(j1, outer, product):
                inner = _collector(lambda q2, v: outer[q2](j1, v))
                for j2 in INNER:
                    inner(j2, product(7 * j1 + j2))
                    yield

            def operands(j1, r):
                _put7(LHS, [_comb(LHS[j1], lambda q1: act[q1, q2, r]) for q2 in range(4)], ab, 7 * j1, r // 2, 0)

            def accumulate(j1, product):
                for j in range(7 * j1, 7 * j1 + 7):
                    acc[t, j] = product(j)
                    yield

            def stages():
                up = [_collector(P(geglu, q2)) for q2 in range(4)]
                out = [_collector(P(store, q2)) for q2 in range(4)]
                down = lambda j: _dot(ab[j], dn[s][j]) if first else acc[t, j] + _dot(ab[j], dn[s][j])
                for ups, downs, ops in (PLAN_LAST if last else PLAN):
                    groups = [products(j1, up, lambda j: _dot(ha[t, j], gu[s][j])) for j1 in ups]
                    groups += [products(j1, out, down) if last else accumulate(j1, down) for j1 in downs]
                    jobs = [P(operands, j1, r) for j1 in ops for r in range(0, Q, 16)]
                    for i in range(7):
                        for g in groups:
                            next(g)
                            yield
                        for job in jobs[len(jobs) * i // 7:len(jobs) * (i + 1) // 7]:
                            job()
            _weave(stages(), 98, sides, lead=lead)

        def first(t):
            if t == 0:
                _start(cp_f(2, 0))
            ffn(0, t, [prep_ffn(1, t) if t else [], span(ln2, Q, 16, L2C, 4 * NT + t)], first=True, lead=first_lead)
        for t in range(peel):
            with scope(f'first{t}'):
                pl.when(go[0] > 0)(P(first, t))
        if peel < NT:
            with scope('firstL'):
                lax.fori_loop(peel, NT, lambda t, _: ffn(0, t, [prep_ffn(1, t)], first=True), None)

        def chunk(c, s):
            def body(i, _):
                for u in range(unroll):
                    ffn(s, i * unroll + u, [prep_ffn(1 - s, i * unroll + u)])
            _wait(cp_f(c + 1, 1 - s))
            pl.when(c + 2 < NF)(lambda: _start(cp_f(c + 2, s)))
            lax.fori_loop(0, NT // unroll, body, None)

        def pair(p, _):
            chunk(2 * p + 1, 1)
            pl.when(p < NF // 2 - 1)(lambda: chunk(2 * p + 2, 0))

        with scope('ffn'):
            lax.fori_loop(0, NF // 2, pair, None)
        with scope('fin'):
            lax.fori_loop(0, NT, lambda t, _: ffn(0, t, [], last=True), None)
        copy(xb, o_hbm, so).wait()

    def fn(A_x, A_wqkv, A_wo, B_x, B_w_gate, B_w_up, B_w_down):
        hbm = pl.BlockSpec(memory_space=pl.ANY)
        V, DMA = pltpu.VMEM, pltpu.SemaphoreType.DMA
        out = pl.pallas_call(
            kernel, in_specs=[hbm] * 6, out_specs=hbm,
            out_shape=jax.ShapeDtypeStruct((S, D), BF16),
            scratch_shapes=(
                [V((S, D), BF16), V((2, D, D), BF16)] + [V((7, D // 4, D // 2), U32)] * 3
                + [V((NH * PITCH, 128), U32)] * 2 + [V((7, H // 2, D // 2), U32)] * NT
                + [V((NCB, S, 128), F32)] + [V((NCB, HALO + S, 128), F32)] * 2
                + [V((NT, 49, Q // 2, D // 4), U32), V((49, Q // 2, FC // 4), U32), V((NT, 49, Q, D // 4), F32)]
                + [V((D, FC), BF16), V((D, FC), BF16), V((FC, D), BF16),
                   V((49, D // 8, FC // 2), U32), V((49, FC // 8, D // 4), U32)] * 2
                + [DMA((7,)), DMA((11,)), DMA((6,)), DMA(()), pltpu.SMEM((1,), jnp.int32)]),
            compiler_params=pltpu.CompilerParams(vmem_limit_bytes=122 * 2 ** 20, flags=flags),
        )(A_x.reshape(S, D), A_wqkv, A_wo, B_w_gate, B_w_up, B_w_down)
        return out.reshape(1, S, D)
    return fn


_impl = make()


@jax.jit
def pallas_sequential_preLN__sliding_local_dilated__glu_gated_geglu__prompt_kernel(
    A_x, A_wqkv, A_wo, B_x, B_w_gate, B_w_up, B_w_down
):
    return _impl(A_x, A_wqkv, A_wo, B_x, B_w_gate, B_w_up, B_w_down)
```

```python
import contextlib
import functools

import jax
import jax.experimental.pallas as pl
import jax.experimental.pallas.tpu as pltpu
import jax.numpy as jnp
import numpy as np
from jax import lax

S, D, F = 2048, 1024, 3584
NH, DH, WIN, DIL = 32, 32, 8, 2
TM, FC = 512, 512
NT, NF = S // TM, F // FC
H, Q = TM // 2, TM // 4
NCB = D // 128
HALO = 16
PITCH = DH + 1
F32, BF16, U32 = jnp.float32, jnp.bfloat16, jnp.uint32
LOG2E = float(np.log2(np.e))
G0 = float(np.sqrt(2.0 / np.pi))
G1 = G0 * 0.044715
P = functools.partial

LHS = (((0, 1), (3, 1)), ((2, 1), (3, 1)), ((0, 1),), ((3, 1),), ((0, 1), (1, 1)), ((2, 1), (0, -1)), ((1, 1), (3, -1)))
RHS = (((0, 1), (3, 1)), ((0, 1),), ((1, 1), (3, -1)), ((2, 1), (0, -1)), ((3, 1),), ((0, 1), (1, 1)), ((2, 1), (3, 1)))
OUT = (((0, 1), (3, 1), (4, -1), (6, 1)), ((2, 1), (4, 1)), ((1, 1), (3, 1)), ((0, 1), (1, -1), (2, 1), (5, 1)))


def _comb(terms, get):
    v = get(terms[0][0])
    for i, sign in terms[1:]:
        a, b = v.astype(F32), get(i).astype(F32)
        v = a + b if sign > 0 else a - b
    return v


def _collector(emit):
    part = {}

    def push(j, val):
        for q, terms in enumerate(OUT):
            sign = dict(terms).get(j)
            if sign is None:
                continue
            if q not in part:
                part[q] = (val, sign, 1)
                continue
            v, s, n = part[q]
            v = v + val if s == sign else v - val if s > 0 else val - v
            part[q] = (v, 1, n + 1)
            if n + 1 == len(terms):
                emit(q, v)
    return push


def _block(q1, q2):
    return 2 * (q1 // 2) + q2 // 2, 2 * (q1 % 2) + q2 % 2


def _cols(c, n=128):
    return pl.ds(c * n, n)


def _ds(start, n, align):
    return pl.ds(start if isinstance(start, int) else pl.multiple_of(start, align), n)


def _bf(v):
    return pltpu.bitcast(v, BF16)


def _dot(a, b):
    return jnp.dot(_bf(a), _bf(b), preferred_element_type=F32)


def _put7(table, quads, dst, base, pair, col):
    for j, terms in enumerate(table):
        v = _comb(terms, quads.__getitem__).astype(BF16)
        dst.at[base + j][_ds(pair, 8, 8), _cols(col)] = pltpu.bitcast(v, U32)


def _weave(main, n, sides, lead=1):
    done = [0] * len(sides)
    for k in range(n):
        next(main)
        for s, side in enumerate(sides):
            upto = min(len(side), -(-len(side) * (k + 1) // (n - lead)))
            for job in side[done[s]:upto]:
                job()
            done[s] = upto


def _start(copies):
    for c in copies:
        c.start()


def _wait(copies):
    for c in copies:
        c.wait()


def make(PM={9: 64, 10: 64, 11: 64, 12: 64},
         BL=128, L1C={-1: 1.5, 0: 2, 1: 2, 2: 3.375, 3: 3.75, 4: 4},
         PRC={3: .6875, 4: 1.375, 5: 2, 6: 2.625, 7: 3, 8: 4},
         PVC={9: 1, 10: 2, 11: 3, 12: 4},
         L2C={13: 1, 14: 2, 15: 3, 16: 4},
         FPC={9: 1, 10: 1.5, 11: 2.5, 12: 4}, F1K=11,
         unroll=1, ahead=3, ffn_lead=3, first_lead=3, peel=1, oloop=0, late=6, PRW={9: (0,), 10: (1, 2), 11: (3,)}, prio=0, LAG=(0, 0, 0, 16), frm=0, boot=0, PROJ=(1, 3, 6, 4, 2, 0, 5), INNER=(1, 3, 6, 4, 2, 0, 5), plan='0 4 6 3 1//2 2//5 5//4 /2/3 /5/1 /4/6 /3/0 /1 /6 /0', last='0 1 2 5 3//3 4//1 6//6 /3/2 /1/4 /6/0 /2/5 /4 /0 /5', cache=True, LP=2, scopes=False, skip=(), upto=16,
         flags={'XLA_TPU_EVENLY_DISTRIBUTE_CRITICAL_NODES': True}):
    PLAN, PLAN_LAST = ([[[int(c) for c in f] for f in (w + '//').split('/')[:3]] for w in p.split()] for p in (plan, last))
    _start = lambda cs: [c.start(priority=prio) for c in cs] and None
    scope = jax.named_scope if scopes else (lambda n: contextlib.nullcontext())

    def kernel(x_hbm, wqkv_hbm, wo_hbm, wg_hbm, wu_hbm, wd_hbm, o_hbm,
               xb, wraw, wp0, wp1, wp2, tmpa, tmpb, tmp1, xa, qb, kb, vb, ha, ab, acc,
               rg, ru, rd, gu0, dn0, gu1, dn1, sx, sw, sf, so, go):
        wp = (wp0, wp1, wp2, wp0)
        gu, dn = (gu0, gu1), (dn0, dn1)
        copy = pltpu.make_async_copy

        def cp_x0(t, i):
            return [copy(x_hbm.at[pl.ds(r, Q)], xb.at[pl.ds(r, Q)], sx.at[r // Q]) for r in (t * TM + i * Q, t * TM + H + i * Q)]

        def cp_x(t):
            return [copy(x_hbm.at[pl.ds(t * TM, TM)], xb.at[pl.ds(t * TM, TM)], sx.at[6 + t])]

        def cp_q(i):
            return [copy(wqkv_hbm.at[pl.ds(r, 128), pl.ds(0, D)], wraw.at[0, pl.ds(r, 128)], sw.at[r // 128])
                    for r in (i * 128, D // 2 + i * 128)]

        def cp_w(m):
            return [copy(wqkv_hbm.at[:, pl.ds(m * D, D)] if m < 3 else wo_hbm, wraw.at[m % 2], sw.at[7 + m])]

        def cp_f(c, s):
            o = _ds(c * FC, FC, FC)
            return [copy(src, dst, sf.at[3 * s + i])
                    for i, (src, dst) in enumerate(zip((wg_hbm.at[:, o], wu_hbm.at[:, o], wd_hbm.at[o]), (rg.at[s], ru.at[s], rd.at[s])))]

        def layernorm(load, parts, finish, lo, hi, lag=16):
            st = {}

            def mean(r, *parts):
                for p in parts:
                    st[r, p] = jnp.sum(load(p + r).sum(0), axis=-1, keepdims=True) * (1.0 / D)

            def rstd(r, *parts):
                for p in parts:
                    xc = load(p + r) - st[r, p]
                    st[r, p, 1] = lax.rsqrt(jnp.sum((xc * xc).sum(0), axis=-1, keepdims=True) * (1.0 / D) + 1e-5)

            jobs = []
            for r in range(lo, hi + 2 * lag, 16):
                jobs += [P(mean, r, *parts[i:i + 2]) for i in range(0, len(parts), 2)] if r < hi else []
                jobs += [P(rstd, r - lag, *parts[i:i + 2]) for i in range(0, len(parts), 2)] if lo <= r - lag < hi else []
                if r - 2 * lag >= lo:
                    jobs += finish(r - 2 * lag, lambda r, p, c: (load(p + r, c) - st[r, p]) * st[r, p, 1])
            return jobs

        def ln1(t, lo, hi):
            def load(r, c=None):
                get = lambda c: xb[pl.ds(t * TM + r, 16), _cols(c)].astype(F32)
                return jnp.stack([get(c) for c in range(NCB)]) if c is None else get(c)

            def put(r, c, norm):
                _put7(LHS, [norm(r, q // 2 * H, q % 2 * 4 + c) for q in range(4)], xa.at[t], 0, r // 2, c)
            return layernorm(load, (0, H), lambda r, norm: [P(put, r, c, norm) for c in range(4)], lo, hi)

        def ln2(t, lo, hi):
            def load(r, c=slice(None)):
                return qb[c, _ds(t * TM + r, 16, 16), :]

            def finish(r, norm):
                @(functools.cache if cache else lambda f: f)
                def get(c, q1, q2):
                    i, k = _block(q1, q2)
                    return norm(r, i * Q, 2 * k + c)

                def put(c, j):
                    _put7(LHS, [_comb(LHS[j], lambda q1: get(c, q1, q2)) for q2 in range(4)], ha.at[t], 7 * j, r // 2, c)
                return [P(put, c, j) for c in range(2) for j in range(7)]
            return layernorm(load, (0, Q, 2 * Q, 3 * Q), finish, lo, hi, LAG[t] if isinstance(t, int) else 0)

        def prep_cols(m, i):
            tmp0 = (tmpa, tmpb)[i % 2]

            def fwd(c):
                w = jnp.concatenate([wraw[m % 2, pl.ds(b + i * 128, 128), _cols(c)] for b in (0, D // 2)], axis=0)
                wt = pltpu.bitcast(w, U32).T
                for h in range(4):
                    tmp0[pl.ds((4 * c + h) * PITCH, DH), :] = wt[h * DH:(h + 1) * DH]

            def back(c):
                rows = [tmp0[pl.ds(4 * c + d, NH, stride=PITCH), :] for d in range(4)]
                tmp1[_cols(c), :] = jnp.concatenate(rows, axis=0).T

            def put(c, r0):
                for r in range(r0, r0 + 32, 8):
                    quads = [_bf(tmp1[pl.ds((q % 2 * 4 + c) * 128 + q // 2 * 64 + r, 8), :]) for q in range(4)]
                    _put7(RHS, quads, wp[m], 0, i * 64 + r, c)
            return ([P(fwd, c) for c in range(NCB)] + [P(back, c) for c in (0, 4, 1, 5, 2, 6, 3, 7)]
                    + [P(put, c, r) for c in range(4) for r in (0, 32)])

        def prep_rows(i):
            def fwd(n, h0):
                for h in range(h0, h0 + 2):
                    w = wraw[1, pl.ds(h * DH, DH), _cols(4 * n + i)].astype(F32)
                    (tmpa, tmpb)[n][pl.ds(h * PITCH, DH), :] = pltpu.bitcast(w, U32)

            def put(d):
                for h in (0, 16):
                    quads = [(tmpa, tmpb)[q % 2][pl.ds(h * PITCH + q // 2 * 16 + d, 16, stride=PITCH), :] for q in range(4)]
                    _put7(RHS, [pltpu.bitcast(v, F32) for v in quads], wp[3], 0, d * 16 + h // 2, i)
            return [P(fwd, n, h) for n in range(2) for h in range(0, NH, 2)] + [P(put, d) for d in range(16)]

        def prep_ffn(s, t, lo=0, hi=84):
            def put(src, dst, kb_, nb, r, c, col, j):
                def get(q1, q2):
                    k, n = _block(q1, q2)
                    return src[_ds(k * kb_ + t * (kb_ // NT) + r, 16, 16), pl.ds(n * nb + c * 128, 128)]
                quads = [_comb(RHS[j], lambda q1: get(q1, q2)) for q2 in range(4)]
                _put7(RHS, quads, dst, 7 * j, t * (kb_ // NT // 2) + r // 2, col)
            jobs = [P(put, (rg, ru)[i].at[s], gu[s], D // 4, FC // 4, r, 0, i, j)
                    for i in range(2) for r in range(0, D // 4 // NT, 16) for j in range(7)]
            jobs += [P(put, rd.at[s], dn[s], FC // 4, D // 4, r, c, c, j)
                     for c in range(2) for r in range(0, FC // 4 // NT, 16) for j in range(7)]
            return jobs[lo:hi]

        def probs(t, lo, hi):
            st = {}

            def dots(r, w):
                k = kb[:, pl.ds(t * TM + r + HALO - DIL * w, 8), :]
                for rr, ww in ((r, w), (r + 8, w + 8 // DIL)):
                    if lo <= rr < hi:
                        st[rr, ww] = (qb[:, pl.ds(t * TM + rr, 8), :] * k).sum(0)

            def fold(r):
                l = jnp.concatenate([st[r, w] for w in range(WIN)], axis=0)
                st[r] = l + pltpu.roll(l, 64, 1)

            def softmax(r):
                l = (st[r] + pltpu.roll(st[r], 32, 1)) * (DH ** -0.5 * LOG2E)
                l = l.reshape(WIN, 8, 128)
                if t * TM + r < DIL * (WIN - 1):
                    pos = t * TM + r + lax.broadcasted_iota(jnp.int32, l.shape, 1)
                    l = jnp.where(pos >= DIL * lax.broadcasted_iota(jnp.int32, l.shape, 0), l, -1e9 * LOG2E)
                p = jnp.exp2(l - l.max(0))
                qb[:, pl.ds(t * TM + r, 8), :] = p * (1.0 / p.sum(0))

            jobs = [P(dots, lo - 8, w) for w in range(4)]
            for r in range(lo, hi, 8):
                jobs += [P(dots, r, w) for w in range(4)] + [P(fold, r)] + ([P(softmax, r - 8)] if r > lo else [])
            return jobs + [P(softmax, hi - 8)]

        def mix(t, lo, hi):
            st = {}

            def part(r, c, i):
                r0 = t * TM + i * H + r
                for w in range(WIN):
                    pv = qb[w, pl.ds(r0, 16), :] * vb[pl.ds(2 * c, 2), pl.ds(r0 + HALO - DIL * w, 16), :]
                    st[i] = st[i] + pv if w else pv
                if i:
                    _put7(LHS, [st[q // 2][q % 2] for q in range(4)], xa.at[t], 0, r // 2, c)
            return [P(part, r, c, i) for r in range(lo, hi, 16) for c in range(4) for i in range(2)]

        def span(fn, size, unit, cuts, k):
            lo, hi = (int(round(cuts.get(i, 0 if i < min(cuts) else NT) * size / unit)) * unit for i in (k - 1, k))
            jobs = []
            for t in range(NT):
                a, b = max(lo - t * size, 0), min(hi - t * size, size)
                jobs += fn(t, a, b) if a < b else []
            return jobs

        def project(m, t, rows, lo, hi, sides):
            def stages():
                for n in range(4):
                    for r in range(lo, hi, rows):
                        def emit(q, val):
                            r0, c = t * TM + q // 2 * H + r, q % 2 * 4 + n
                            if m == 0:
                                qb[c, pl.ds(r0, rows), :] = val
                            elif m == 1:
                                kb[c, pl.ds(HALO + r0, rows), :] = val
                            elif m == 2:
                                vb[2 * n + q % 2, pl.ds(HALO + r0, rows), :] = val
                            else:
                                qb[c, _ds(r0, rows, rows), :] = val + xb[_ds(r0, rows, rows), _cols(c)].astype(F32)
                        push = _collector(emit)
                        for j in PROJ:
                            push(j, _dot(xa[t, j, pl.ds(r // 2, rows // 2), :], wp[m][j, :, _cols(n)]))
                            yield
            n = (hi - lo) // rows
            _weave(stages(), 28 * n, sides, lead=n)

        def zipped(*lists):
            return [job for _, job in sorted(((n / len(l), job) for l in lists for n, job in enumerate(l)), key=lambda e: e[0])]

        head = prep_cols(0, 0)
        go[0] = 1
        _start(cp_x0(0, 0) + cp_q(0))
        kb[:, pl.ds(0, HALO), :] = jnp.zeros((NCB, HALO, 128), F32)
        for i, (now, later, jobs) in enumerate(((cp_x0(0, 0), cp_x0(0, 1), ln1(0, 0, Q)),
                                                (cp_q(0), cp_q(1), head[:2 * NCB]),
                                                (cp_x0(0, 1), cp_q(2), zipped(head[2 * NCB:], ln1(0, Q, H))))):
            with scope(f'w{i}'):
                _wait(now)
            _start(later)
            for job in jobs:
                job()

        def boot(i):
            if i or not late:
                _wait(cp_q(i + 1) if i < 3 else cp_x0(1, 0))
            pre = [lambda: None] * late + [lambda: _wait(cp_q(1))] if late and not i else []
            _start((P(cp_q, 3), P(cp_x0, 1, 0), P(cp_x0, 1, 1), P(cp_w, 1))[i]())

            def stages():
                for r in range(2):
                    for n in range(2):
                        def emit(q, val):
                            for c in range(2):
                                qb[q % 2 * 4 + 2 * n + c, pl.ds(q // 2 * H + r * Q, Q), :] = val[:, c * 128:(c + 1) * 128]
                        push = _collector(emit)
                        for j in PROJ:
                            val = _dot(xa[0, j, pl.ds(r * Q // 2, Q // 2), _cols(i)], wp0[j, pl.ds(i * 64, 64), _cols(n, 256)])
                            val = val + acc[2 * r + n, j] if i else val
                            if i < 3:
                                acc[2 * r + n, j] = val
                            else:
                                push(j, val)
                            yield
            _weave(stages(), 28, [pre + prep_cols(0, i + 1) if i < 3 else ln1(1, 0, BL)], lead=2)
        for i in range(4):
            with scope(f'boot{i}'):
                pl.when(go[0] > 0)(P(boot, i))

        order = ((0, 1), (0, 1), (1, 0), (1, 1), (0, 2), (1, 2), (0, 3), (1, 3)) + tuple((m, t) for m in (2, 3) for t in range(NT))

        def step(k):
            sides = []
            if k == 0:
                _wait(cp_x0(1, 1))
                _start(cp_x(2))
            elif k == 1:
                _wait(cp_w(1))
                _start(cp_x(3))
                sides.append(sum((prep_cols(1, i) for i in range(4)), []))
            elif k == 2:
                _wait(cp_x(2) + cp_x(3))
                _start(cp_w(2) + cp_f(0, 0))
            elif k == 3:
                _start(cp_w(3))
            elif k == 4:
                _wait(cp_w(2))
                _start(cp_f(1, 1))
            elif k == 7:
                _wait(cp_w(3) + cp_f(0, 0) + cp_f(1, 1))
            elif k == 9:
                vb[:, pl.ds(0, HALO), :] = jnp.broadcast_to(vb[:, pl.ds(HALO, 1), :], (NCB, HALO, 128))
            if 4 <= k < 12:
                sides.append((prep_cols(2, k - 4) if k < 8 else []) + sum((prep_rows(i) for i in PRW.get(k, ())), []))
            sides = [span(ln1, H, 16, L1C, k), span(probs, TM, 8, PRC, k), span(mix, H, 16, PVC, k)] + sides + [
                span(P(prep_ffn, 0), 84, 1, FPC, k), span(ln2, Q, 16, L2C, k)]
            if k == F1K:
                sides.append(prep_ffn(1, 0))
            if frm <= k < upto:
                project(*order[k], *(((BL, 0, BL), (BL, BL, H))[k] if k < 2 else (PM.get(k, H), 0, H)), sides)

        for k in range(4 * NT - 3 * oloop):
            with scope(f'step{k:02d}'):
                pl.when(go[0] > 0)(P(step, k))
        if oloop:
            with scope('oloop'):
                lax.fori_loop(1, NT, lambda t, _: project(3, t, PM.get(13, H), 0, H, [ln2(t - 1, 0, Q)]), None)

        def ffn(s, t, sides, first=False, last=False, lead=ffn_lead):
            act = {}

            def geglu(q2, q1, val):
                for r in range(0, Q, 16):
                    g, u = val[r:r + 16, :128], val[r:r + 16, 128:]
                    act[q1, q2, r] = (g * u) * (jnp.tanh(g * (g * g * G1 + G0)) * 0.5 + 0.5)

            def store(q2, q1, val):
                i, n = _block(q1, q2)
                rows = _ds(t * TM + i * Q, Q, Q)
                for c in range(2):
                    xb[rows, _cols(2 * n + c)] = (qb[2 * n + c, rows, :] + val[:, c * 128:(c + 1) * 128]).astype(BF16)
                copy(xb.at[rows, _cols(n, 256)], o_hbm.at[rows, _cols(n, 256)], so).start()

            def products(j1, outer, product):
                inner = _collector(lambda q2, v: outer[q2](j1, v))
                for j2 in INNER:
                    inner(j2, product(7 * j1 + j2))
                    yield

            def operands(j1, r):
                _put7(LHS, [_comb(LHS[j1], lambda q1: act[q1, q2, r]) for q2 in range(4)], ab, 7 * j1, r // 2, 0)

            def accumulate(j1, product):
                for j in range(7 * j1, 7 * j1 + 7):
                    acc[t, j] = product(j)
                    yield

            def stages():
                up = [_collector(P(geglu, q2)) for q2 in range(4)]
                out = [_collector(P(store, q2)) for q2 in range(4)]
                down = lambda j: _dot(ab[j], dn[s][j]) if first else acc[t, j] + _dot(ab[j], dn[s][j])
                for ups, downs, ops in (PLAN_LAST if last else PLAN):
                    groups = [products(j1, up, lambda j: _dot(ha[t, j], gu[s][j])) for j1 in ups]
                    groups += [products(j1, out, down) if last else accumulate(j1, down) for j1 in downs]
                    jobs = [P(operands, j1, r) for j1 in ops for r in range(0, Q, 16)]
                    for i in range(7):
                        for g in groups:
                            next(g)
                            yield
                        for job in jobs[len(jobs) * i // 7:len(jobs) * (i + 1) // 7]:
                            job()
            _weave(stages(), 98, sides, lead=lead)

        def first(t):
            if t == 0:
                _start(cp_f(2, 0))
            ffn(0, t, [prep_ffn(1, t) if t else [], span(ln2, Q, 16, L2C, 4 * NT + t)], first=True, lead=first_lead)
        for t in range(peel):
            with scope(f'first{t}'):
                pl.when(go[0] > 0)(P(first, t))
        if peel < NT:
            with scope('firstL'):
                lax.fori_loop(peel, NT, lambda t, _: ffn(0, t, [prep_ffn(1, t)], first=True), None)

        def chunk(c, s):
            def body(i, _):
                for u in range(unroll):
                    ffn(s, i * unroll + u, [prep_ffn(1 - s, i * unroll + u)])
            _wait(cp_f(c + 1, 1 - s))
            pl.when(c + 2 < NF)(lambda: _start(cp_f(c + 2, s)))
            lax.fori_loop(0, NT // unroll, body, None)

        def pair(p, _):
            chunk(2 * p + 1, 1)
            pl.when(p < NF // 2 - 1)(lambda: chunk(2 * p + 2, 0))

        with scope('ffn'):
            lax.fori_loop(0, NF // 2, pair, None)
        with scope('fin'):
            lax.fori_loop(0, NT, lambda t, _: ffn(0, t, [], last=True), None)
        copy(xb, o_hbm, so).wait()

    def fn(A_x, A_wqkv, A_wo, B_x, B_w_gate, B_w_up, B_w_down):
        hbm = pl.BlockSpec(memory_space=pl.ANY)
        V, DMA = pltpu.VMEM, pltpu.SemaphoreType.DMA
        out = pl.pallas_call(
            kernel, in_specs=[hbm] * 6, out_specs=hbm,
            out_shape=jax.ShapeDtypeStruct((S, D), BF16),
            scratch_shapes=(
                [V((S, D), BF16), V((2, D, D), BF16)] + [V((7, D // 4, D // 2), U32)] * 3
                + [V((NH * PITCH, 128), U32)] * 3 + [V((NT, 7, H // 2, D // 2), U32)]
                + [V((NCB, S, 128), F32)] + [V((NCB, HALO + S, 128), F32)] * 2
                + [V((NT, 49, Q // 2, D // 4), U32), V((49, Q // 2, FC // 4), U32), V((NT, 49, Q, D // 4), F32)]
                + [V((2, D, FC), BF16), V((2, D, FC), BF16), V((2, FC, D), BF16)]
                + [V((49, D // 8, FC // 2), U32), V((49, FC // 8, D // 4), U32)] * 2
                + [DMA((10,)), DMA((11,)), DMA((6,)), DMA(()), pltpu.SMEM((1,), jnp.int32)]),
            compiler_params=pltpu.CompilerParams(vmem_limit_bytes=122 * 2 ** 20, flags=flags),
        )(A_x.reshape(S, D), A_wqkv, A_wo, B_w_gate, B_w_up, B_w_down)
        return out.reshape(1, S, D)
    return fn


_impl = make()


@jax.jit
def pallas_sequential_preLN__sliding_local_dilated__glu_gated_geglu__prompt_kernel(
    A_x, A_wqkv, A_wo, B_x, B_w_gate, B_w_up, B_w_down
):
    return _impl(A_x, A_wqkv, A_wo, B_x, B_w_gate, B_w_up, B_w_down)
```

```python
import functools

import jax
import jax.experimental.pallas as pl
import jax.experimental.pallas.tpu as pltpu
import jax.numpy as jnp
import numpy as np
from jax import lax

S, D, F = 2048, 1024, 3584
NH, DH, WIN, DIL = 32, 32, 8, 2
TM, FC = 512, 512
NT, NF = S // TM, F // FC
H, Q = TM // 2, TM // 4
NCB = D // 128
HALO = 16
PITCH = DH + 1
F32, BF16, U32 = jnp.float32, jnp.bfloat16, jnp.uint32
LOG2E = float(np.log2(np.e))
G0 = float(np.sqrt(2.0 / np.pi))
G1 = G0 * 0.044715
P = functools.partial

LHS = (((0, 1), (3, 1)), ((2, 1), (3, 1)), ((0, 1),), ((3, 1),), ((0, 1), (1, 1)), ((2, 1), (0, -1)), ((1, 1), (3, -1)))
RHS = (((0, 1), (3, 1)), ((0, 1),), ((1, 1), (3, -1)), ((2, 1), (0, -1)), ((3, 1),), ((0, 1), (1, 1)), ((2, 1), (3, 1)))
OUT = ({0: 1, 3: 1, 4: -1, 6: 1}, {2: 1, 4: 1}, {1: 1, 3: 1}, {0: 1, 1: -1, 2: 1, 5: 1})

PROJ_ORDER = (1, 3, 6, 4, 2, 0, 5)
UP_ORDER = (1, 3, 2, 4, 0, 5, 6)
DOWN_ORDER = (5, 1, 3, 0, 2, 4, 6)
FFN_PLAN = ((0, 4, 6, 3, 1, 2, 5), (2, 5, 4, 3, 1, 6, 0))
FFN_PLAN_LAST = ((0, 1, 2, 5, 3, 4, 6), (3, 1, 6, 2, 4, 0, 5))

STEPS = ((0, 1, Q, 0, Q), (0, 1, Q, Q, H), (1, 0, H, 0, H), (1, 1, H, 0, H),
         (0, 2, H, 0, H), (1, 2, H, 0, H), (0, 3, H, 0, H), (1, 3, H, 0, H),
         (2, 0, H, 0, H), (2, 1, 64, 0, H), (2, 2, 64, 0, H), (2, 3, 64, 0, H),
         (3, 0, 64, 0, H), (3, 1, H, 0, H), (3, 2, H, 0, H), (3, 3, H, 0, H))
LN1_DONE = {-1: 1.5, 0: 2, 1: 2, 2: 3.375, 3: 3.75, 4: 4}
PROBS_DONE = {3: 0.6875, 4: 1.375, 5: 2, 6: 2.625, 7: 3, 8: 4}
MIX_DONE = {9: 1, 10: 2, 11: 3, 12: 4}
LN2_DONE = {13: 1, 14: 2, 15: 3}
FFN0_DONE = {9: 1, 10: 1.5, 11: 2.5, 12: 4}
WO_PARTS = {9: (0,), 10: (1, 2), 11: (3,)}


def _comb(terms, get):
    v = get(terms[0][0])
    for i, sign in terms[1:]:
        a, b = v.astype(F32), get(i).astype(F32)
        v = a + b if sign > 0 else a - b
    return v


def _collector(emit):
    part = {}

    def push(j, val):
        for q, terms in enumerate(OUT):
            if j not in terms:
                continue
            if q not in part:
                part[q] = (val, terms[j], 1)
                continue
            v, sign, n = part[q]
            v = v + val if sign == terms[j] else v - val if sign > 0 else val - v
            part[q] = (v, 1, n + 1)
            if n + 1 == len(terms):
                emit(q, v)
    return push


def _block(q1, q2):
    return 2 * (q1 // 2) + q2 // 2, 2 * (q1 % 2) + q2 % 2


def _cols(c, n=128):
    return pl.ds(c * n, n)


def _ds(start, n):
    return pl.ds(start if isinstance(start, int) else pl.multiple_of(start, n), n)


def _dot(a, b):
    return jnp.dot(pltpu.bitcast(a, BF16), pltpu.bitcast(b, BF16), preferred_element_type=F32)


def _put7(table, quads, dst, pair, col, base=0):
    for j, terms in enumerate(table):
        v = _comb(terms, lambda q: quads[q]).astype(BF16)
        dst.at[base + j][_ds(pair, 8), _cols(col)] = pltpu.bitcast(v, U32)


def _put49(table, get, dst, pair, col, j):
    quads = [_comb(table[j], lambda q1: get(*_block(q1, q2))) for q2 in range(4)]
    _put7(table, quads, dst, pair, col, 7 * j)


def _weave(main, n, sides, lead):
    done = [0] * len(sides)
    for k in range(n):
        next(main)
        for s, side in enumerate(sides):
            upto = min(len(side), -(-len(side) * (k + 1) // (n - lead)))
            for job in side[done[s]:upto]:
                job()
            done[s] = upto


def _span(fn, size, unit, done, k):
    if k not in done:
        return []
    lo, hi = (int(round(done.get(i, 0) * size / unit)) * unit for i in (k - 1, k))
    jobs = []
    for t in range(NT):
        a, b = max(lo - t * size, 0), min(hi - t * size, size)
        jobs += fn(t, a, b) if a < b else []
    return jobs


def _start(copies):
    for c in copies:
        c.start()


def _wait(copies):
    for c in copies:
        c.wait()


def _kernel(x_hbm, wqkv_hbm, wo_hbm, wg_hbm, wu_hbm, wd_hbm, o_hbm,
            xb, wraw, wp0, wp1, wp2, tmpa, tmpb, tmpc, xa, qb, kb, vb, ha, ab, acc,
            rg, ru, rd, gu0, dn0, gu1, dn1, sx, sw, sf, so, go):
    wp = (wp0, wp1, wp2, wp0)
    gu, dn = (gu0, gu1), (dn0, dn1)
    copy = pltpu.make_async_copy

    def block(fn):
        pl.when(go[0] > 0)(fn)

    def cp_x_half(t, i):
        return [copy(x_hbm.at[pl.ds(r, Q)], xb.at[pl.ds(r, Q)], sx.at[r // Q])
                for r in (t * TM + i * Q, t * TM + H + i * Q)]

    def cp_x(t):
        return [copy(x_hbm.at[pl.ds(t * TM, TM)], xb.at[pl.ds(t * TM, TM)], sx.at[6 + t])]

    def cp_wq(i):
        return [copy(wqkv_hbm.at[pl.ds(r, 128), pl.ds(0, D)], wraw.at[0, pl.ds(r, 128)], sw.at[r // 128])
                for r in (i * 128, D // 2 + i * 128)]

    def cp_w(m):
        return [copy(wqkv_hbm.at[:, pl.ds(m * D, D)] if m < 3 else wo_hbm, wraw.at[m % 2], sw.at[7 + m])]

    def cp_ffn(c, s):
        o = _ds(c * FC, FC)
        pairs = ((wg_hbm.at[:, o], rg), (wu_hbm.at[:, o], ru), (wd_hbm.at[o], rd))
        return [copy(src, dst.at[s], sf.at[3 * s + i]) for i, (src, dst) in enumerate(pairs)]

    def layernorm(load, parts, finish, lo, hi, lag):
        mu, rs = {}, {}

        def mean(*rows):
            for r in rows:
                mu[r] = jnp.sum(load(r).sum(0), axis=-1, keepdims=True) * (1.0 / D)

        def rstd(*rows):
            for r in rows:
                xc = load(r) - mu[r]
                rs[r] = lax.rsqrt(jnp.sum((xc * xc).sum(0), axis=-1, keepdims=True) * (1.0 / D) + 1e-5)

        jobs = []
        for r in range(lo, hi + 2 * lag, 16):
            for fn, rr in ((mean, r), (rstd, r - lag)):
                if lo <= rr < hi:
                    jobs += [P(fn, rr + parts[i], rr + parts[i + 1]) for i in range(0, len(parts), 2)]
            if r - 2 * lag >= lo:
                jobs += finish(r - 2 * lag, lambda r, c: (load(r, c) - mu[r]) * rs[r])
        return jobs

    def ln1(t, lo, hi):
        def load(r, c=None):
            if c is None:
                return jnp.stack([load(r, c) for c in range(NCB)])
            return xb[pl.ds(t * TM + r, 16), _cols(c)].astype(F32)

        def put(r, c, norm):
            _put7(LHS, [norm(r + q // 2 * H, q % 2 * 4 + c) for q in range(4)], xa.at[t], r // 2, c)
        return layernorm(load, (0, H), lambda r, norm: [P(put, r, c, norm) for c in range(4)], lo, hi, 16)

    def ln2(t, lo, hi, lag=0):
        def load(r, c=slice(None)):
            return qb[c, pl.ds(t * TM + r, 16), :]

        def finish(r, norm):
            get = functools.cache(lambda c, i, k: norm(r + i * Q, 2 * k + c))
            return [P(_put49, LHS, P(get, c), ha.at[t], r // 2, c, j) for c in range(2) for j in range(7)]
        return layernorm(load, (0, Q, 2 * Q, 3 * Q), finish, lo, hi, lag)

    def prep_cols(m, i):
        tmp = (tmpa, tmpb)[i % 2]

        def fwd(c):
            w = jnp.concatenate([wraw[m % 2, pl.ds(b + i * 128, 128), _cols(c)] for b in (0, D // 2)], axis=0)
            wt = pltpu.bitcast(w, U32).T
            for h in range(4):
                tmp[pl.ds((4 * c + h) * PITCH, DH), :] = wt[h * DH:(h + 1) * DH]

        def back(c):
            rows = [tmp[pl.ds(4 * c + d, NH, stride=PITCH), :] for d in range(4)]
            tmpc[_cols(c), :] = jnp.concatenate(rows, axis=0).T

        def put(c, r0):
            for r in range(r0, r0 + 32, 8):
                quads = [tmpc[pl.ds((q % 2 * 4 + c) * 128 + q // 2 * 64 + r, 8), :] for q in range(4)]
                _put7(RHS, [pltpu.bitcast(v, BF16) for v in quads], wp[m], i * 64 + r, c)
        return ([P(fwd, c) for c in range(NCB)] + [P(back, c) for c in (0, 4, 1, 5, 2, 6, 3, 7)]
                + [P(put, c, r) for c in range(4) for r in (0, 32)])

    def prep_rows(i):
        def fwd(n, h0):
            for h in (h0, h0 + 1):
                w = wraw[1, pl.ds(h * DH, DH), _cols(4 * n + i)].astype(F32)
                (tmpa, tmpb)[n][pl.ds(h * PITCH, DH), :] = pltpu.bitcast(w, U32)

        def put(d):
            for h in (0, 16):
                quads = [(tmpa, tmpb)[q % 2][pl.ds(h * PITCH + q // 2 * 16 + d, 16, stride=PITCH), :]
                         for q in range(4)]
                _put7(RHS, [pltpu.bitcast(v, F32) for v in quads], wp[3], d * 16 + h // 2, i)
        return [P(fwd, n, h) for n in range(2) for h in range(0, NH, 2)] + [P(put, d) for d in range(16)]

    def prep_ffn(s, t, lo=0, hi=84):
        def part(src, dst, rows, cols, c, col):
            def get(r, k, n):
                return src[s, _ds(k * rows + t * (rows // NT) + r, 16), pl.ds(n * cols + c * 128, 128)]
            return [P(_put49, RHS, P(get, r), dst, t * (rows // NT // 2) + r // 2, col, j)
                    for r in range(0, rows // NT, 16) for j in range(7)]
        jobs = part(rg, gu[s], D // 4, FC // 4, 0, 0) + part(ru, gu[s], D // 4, FC // 4, 0, 1)
        jobs += part(rd, dn[s], FC // 4, D // 4, 0, 0) + part(rd, dn[s], FC // 4, D // 4, 1, 1)
        return jobs[lo:hi]

    def probs(t, lo, hi):
        st = {}

        def dots(r, w):
            k = kb[:, pl.ds(t * TM + r + HALO - DIL * w, 8), :]
            for rr, ww in ((r, w), (r + 8, w + 8 // DIL)):
                if lo <= rr < hi:
                    st[rr, ww] = (qb[:, pl.ds(t * TM + rr, 8), :] * k).sum(0)

        def fold(r):
            l = jnp.concatenate([st[r, w] for w in range(WIN)], axis=0)
            st[r] = l + pltpu.roll(l, 64, 1)

        def softmax(r):
            l = (st[r] + pltpu.roll(st[r], 32, 1)) * (DH ** -0.5 * LOG2E)
            l = l.reshape(WIN, 8, 128)
            if t * TM + r < DIL * (WIN - 1):
                pos = t * TM + r + lax.broadcasted_iota(jnp.int32, l.shape, 1)
                l = jnp.where(pos >= DIL * lax.broadcasted_iota(jnp.int32, l.shape, 0), l, -1e9 * LOG2E)
            p = jnp.exp2(l - l.max(0))
            qb[:, pl.ds(t * TM + r, 8), :] = p * (1.0 / p.sum(0))

        jobs = [P(dots, lo - 8, w) for w in range(4)]
        for r in range(lo, hi, 8):
            jobs += [P(dots, r, w) for w in range(4)] + [P(fold, r)] + ([P(softmax, r - 8)] if r > lo else [])
        return jobs + [P(softmax, hi - 8)]

    def mix(t, lo, hi):
        st = {}

        def part(r, c, i):
            r0 = t * TM + i * H + r
            for w in range(WIN):
                pv = qb[w, pl.ds(r0, 16), :] * vb[pl.ds(2 * c, 2), pl.ds(r0 + HALO - DIL * w, 16), :]
                st[i] = st[i] + pv if w else pv
            if i:
                _put7(LHS, [st[q // 2][q % 2] for q in range(4)], xa.at[t], r // 2, c)
        return [P(part, r, c, i) for r in range(lo, hi, 16) for c in range(4) for i in range(2)]

    head, tail = prep_cols(0, 0), ln1(0, Q, H)
    for n, job in enumerate(head[2 * NCB:]):
        tail.insert(7 * n, job)
    go[0] = 1
    _start(cp_x_half(0, 0) + cp_wq(0))
    kb[:, pl.ds(0, HALO), :] = jnp.zeros((NCB, HALO, 128), F32)
    for now, later, jobs in ((cp_x_half(0, 0), cp_x_half(0, 1), ln1(0, 0, Q)),
                             (cp_wq(0), cp_wq(1), head[:2 * NCB]),
                             (cp_x_half(0, 1), cp_wq(2), tail)):
        _wait(now)
        _start(later)
        for job in jobs:
            job()

    def boot(i):
        if i == 0:
            _start(cp_wq(3))
            sides = [[lambda: None] * 6 + [lambda: _wait(cp_wq(1))] + prep_cols(0, 1)]
        elif i == 1:
            _wait(cp_wq(2))
            _start(cp_x_half(1, 0))
            sides = [prep_cols(0, 2)]
        elif i == 2:
            _wait(cp_wq(3) + cp_x_half(1, 0))
            _start(cp_x_half(1, 1))
            sides = [prep_cols(0, 3), ln1(1, 0, 48)]
        else:
            _start(cp_w(1))
            sides = [ln1(1, 48, Q)]

        def stages():
            for r in range(2):
                for n in range(2):
                    def emit(q, val):
                        for c in range(2):
                            qb[q % 2 * 4 + 2 * n + c, pl.ds(q // 2 * H + r * Q, Q), :] = val[:, c * 128:(c + 1) * 128]
                    push = _collector(emit)
                    for j in PROJ_ORDER:
                        val = _dot(xa[0, j, _cols(r, Q // 2), _cols(i)], wp0[j, _cols(i, 64), _cols(n, 256)])
                        val = val + acc[2 * r + n, j] if i else val
                        if i < 3:
                            acc[2 * r + n, j] = val
                        else:
                            push(j, val)
                        yield
        _weave(stages(), 28, sides, 2)

    def step(k):
        m, t, rows, lo, hi = STEPS[k]
        prep = sum((prep_rows(i) for i in WO_PARTS.get(k, ())), [])
        if k == 0:
            _wait(cp_x_half(1, 1))
            _start(cp_x(2))
        elif k == 1:
            _wait(cp_w(1))
            _start(cp_x(3))
            prep = sum((prep_cols(1, i) for i in range(4)), [])
        elif k == 2:
            _wait(cp_x(2) + cp_x(3))
            _start(cp_w(2) + cp_ffn(0, 0))
        elif k == 3:
            _start(cp_w(3))
        elif k == 4:
            _wait(cp_w(2))
            _start(cp_ffn(1, 1))
        elif k == 7:
            _wait(cp_w(3) + cp_ffn(0, 0) + cp_ffn(1, 1))
        elif k == 9:
            vb[:, pl.ds(0, HALO), :] = jnp.broadcast_to(vb[:, pl.ds(HALO, 1), :], (NCB, HALO, 128))
        if 4 <= k < 8:
            prep = prep_cols(2, k - 4)
        sides = [_span(ln1, H, 16, LN1_DONE, k), _span(probs, TM, 8, PROBS_DONE, k), _span(mix, H, 16, MIX_DONE, k),
                 prep, _span(P(prep_ffn, 0), 84, 1, FFN0_DONE, k), _span(ln2, Q, 16, LN2_DONE, k),
                 prep_ffn(1, 0) if k == 11 else []]

        def stages():
            for n in range(4):
                for r in range(lo, hi, rows):
                    def emit(q, val):
                        r0, c = t * TM + q // 2 * H + r, q % 2 * 4 + n
                        if m == 0:
                            qb[c, pl.ds(r0, rows), :] = val
                        elif m == 1:
                            kb[c, pl.ds(HALO + r0, rows), :] = val
                        elif m == 2:
                            vb[2 * n + q % 2, pl.ds(HALO + r0, rows), :] = val
                        else:
                            qb[c, pl.ds(r0, rows), :] = val + xb[pl.ds(r0, rows), _cols(c)].astype(F32)
                    push = _collector(emit)
                    for j in PROJ_ORDER:
                        push(j, _dot(xa[t, j, pl.ds(r // 2, rows // 2), :], wp[m][j, :, _cols(n)]))
                        yield
        _weave(stages(), 28 * ((hi - lo) // rows), sides, (hi - lo) // rows)

    for i in range(4):
        block(P(boot, i))
    for k in range(len(STEPS)):
        block(P(step, k))

    def ffn(s, t, side, first=False, last=False):
        act = {}

        def geglu(q2, q1, val):
            for r in range(0, Q, 16):
                g, u = val[r:r + 16, :128], val[r:r + 16, 128:]
                act[(r,) + _block(q1, q2)] = (g * u) * (jnp.tanh(g * (g * g * G1 + G0)) * 0.5 + 0.5)

        def store(q2, q1, val):
            i, n = _block(q1, q2)
            rows = _ds(t * TM + i * Q, Q)
            for c in range(2):
                xb[rows, _cols(2 * n + c)] = (qb[2 * n + c, rows, :] + val[:, c * 128:(c + 1) * 128]).astype(BF16)
            copy(xb.at[rows, _cols(n, 256)], o_hbm.at[rows, _cols(n, 256)], so).start()

        def down(j):
            return _dot(ab[j], dn[s][j]) if first else acc[t, j] + _dot(ab[j], dn[s][j])

        def combine(j1, outer, order, product):
            inner = _collector(lambda q2, v: outer[q2](j1, v))
            for j2 in order:
                inner(j2, product(7 * j1 + j2))
                yield

        def accumulate(j1):
            for j in range(7 * j1, 7 * j1 + 7):
                acc[t, j] = down(j)
                yield

        def stages():
            ups, downs = FFN_PLAN_LAST if last else FFN_PLAN
            up = [_collector(P(geglu, q2)) for q2 in range(4)]
            out = [_collector(P(store, q2)) for q2 in range(4)]
            groups = [combine(j1, up, UP_ORDER, lambda j: _dot(ha[t, j], gu[s][j])) for j1 in ups]
            groups += [combine(j1, out, DOWN_ORDER, down) if last else accumulate(j1) for j1 in downs]
            for n, group in enumerate(groups):
                rows = range(0, Q if 4 <= n < 11 else 0, 16)
                for i, _ in enumerate(group):
                    yield
                    for r in rows[len(rows) * i // 7:len(rows) * (i + 1) // 7]:
                        _put49(LHS, lambda a, b: act[r, a, b], ab, r // 2, 0, downs[n - 4])
        _weave(stages(), 98, [side], 3)

    def enter():
        _start(cp_ffn(2, 0))
        ffn(0, 0, ln2(NT - 1, 0, Q, 16), first=True)

    def chunk(c, s):
        _wait(cp_ffn(c + 1, 1 - s))
        pl.when(c + 2 < NF)(lambda: _start(cp_ffn(c + 2, s)))
        lax.fori_loop(0, NT, lambda t, _: ffn(s, t, prep_ffn(1 - s, t)), None)

    def pair(p, _):
        chunk(2 * p + 1, 1)
        pl.when(p < NF // 2 - 1)(lambda: chunk(2 * p + 2, 0))

    block(enter)
    lax.fori_loop(1, NT, lambda t, _: ffn(0, t, prep_ffn(1, t), first=True), None)
    lax.fori_loop(0, NF // 2, pair, None)
    lax.fori_loop(0, NT, lambda t, _: ffn(0, t, [], last=True), None)
    copy(xb, o_hbm, so).wait()


@jax.jit
def pallas_sequential_preLN__sliding_local_dilated__glu_gated_geglu__prompt_kernel(
    A_x: jax.Array,
    A_wqkv: jax.Array,
    A_wo: jax.Array,
    B_x: jax.Array,
    B_w_gate: jax.Array,
    B_w_up: jax.Array,
    B_w_down: jax.Array,
):
    del B_x
    hbm = pl.BlockSpec(memory_space=pl.ANY)
    vmem, dma = pltpu.VMEM, pltpu.SemaphoreType.DMA
    out = pl.pallas_call(
        _kernel,
        in_specs=[hbm] * 6,
        out_specs=hbm,
        out_shape=jax.ShapeDtypeStruct((S, D), BF16),
        scratch_shapes=(
            [vmem((S, D), BF16), vmem((2, D, D), BF16)] + [vmem((7, D // 4, D // 2), U32)] * 3
            + [vmem((NH * PITCH + DH, 128), U32)] * 2 + [vmem((D, 128), U32), vmem((NT, 7, H // 2, D // 2), U32)]
            + [vmem((NCB, S, 128), F32)] + [vmem((NCB, HALO + S, 128), F32)] * 2
            + [vmem((NT, 49, Q // 2, D // 4), U32), vmem((49, Q // 2, FC // 4), U32), vmem((NT, 49, Q, D // 4), F32)]
            + [vmem((2, D, FC), BF16), vmem((2, D, FC), BF16), vmem((2, FC, D), BF16)]
            + [vmem((49, D // 8, FC // 2), U32), vmem((49, FC // 8, D // 4), U32)] * 2
            + [dma((10,)), dma((11,)), dma((6,)), dma(()), pltpu.SMEM((1,), jnp.int32)]),
        compiler_params=pltpu.CompilerParams(
            vmem_limit_bytes=122 * 2 ** 20,
            flags={"XLA_TPU_EVENLY_DISTRIBUTE_CRITICAL_NODES": True},
        ),
    )(A_x.reshape(S, D), A_wqkv, A_wo, B_w_gate, B_w_up, B_w_down)
    return out.reshape(1, S, D)
```

```python
import functools

import jax
import jax.experimental.pallas as pl
import jax.experimental.pallas.tpu as pltpu
import jax.numpy as jnp
import numpy as np
from jax import lax

S, D, F = 2048, 1024, 3584
NH, DH, WIN, DIL = 32, 32, 8, 2
TM, FC = 512, 512
NT, NF = S // TM, F // FC
H, Q = TM // 2, TM // 4
NCB = D // 128
HALO = 16
PITCH = DH + 1
F32, BF16, U32 = jnp.float32, jnp.bfloat16, jnp.uint32
LOG2E = float(np.log2(np.e))
G0 = float(np.sqrt(2.0 / np.pi))
G1 = G0 * 0.044715
P = functools.partial

LHS = (((0, 1), (3, 1)), ((2, 1), (3, 1)), ((0, 1),), ((3, 1),), ((0, 1), (1, 1)), ((2, 1), (0, -1)), ((1, 1), (3, -1)))
RHS = (((0, 1), (3, 1)), ((0, 1),), ((1, 1), (3, -1)), ((2, 1), (0, -1)), ((3, 1),), ((0, 1), (1, 1)), ((2, 1), (3, 1)))
OUT = ({0: 1, 3: 1, 4: -1, 6: 1}, {2: 1, 4: 1}, {1: 1, 3: 1}, {0: 1, 1: -1, 2: 1, 5: 1})

PROJ_ORDER = (1, 3, 6, 4, 2, 0, 5)
UP_ORDER = (1, 3, 2, 4, 0, 5, 6)
DOWN_ORDER = (5, 1, 3, 0, 2, 4, 6)
FFN_PLAN = ((0, 4, 6, 3, 1, 2, 5), (2, 5, 4, 3, 1, 6, 0))
FFN_PLAN_LAST = ((0, 1, 2, 5, 3, 4, 6), (3, 1, 6, 2, 4, 0, 5))

PARKED = {0: (0, 1), 1: (2, 3), 2: (4, 5), 3: (6,)}

STEPS = ((0, 1, Q, 0, Q), (0, 1, Q, Q, H), (1, 0, H, 0, H), (1, 1, H, 0, H),
         (0, 2, H, 0, H), (1, 2, H, 0, H), (0, 3, H, 0, H), (1, 3, H, 0, H),
         (2, 0, H, 0, H), (2, 1, 64, 0, H), (2, 2, 64, 0, H), (2, 3, 64, 0, H),
         (3, 0, 64, 0, H), (3, 1, H, 0, H), (3, 2, H, 0, H), (3, 3, H, 0, H))
LN1_DONE = {-1: 1.5, 0: 2, 1: 2, 2: 3.375, 3: 3.75, 4: 4}
PROBS_DONE = {3: 0.6875, 4: 1.375, 5: 2, 6: 2.625, 7: 3, 8: 4}
MIX_DONE = {9: 1, 10: 2, 11: 3, 12: 4}
LN2_DONE = {13: 1, 14: 2, 15: 3}
FFN0_DONE = {9: 1, 10: 1.5, 11: 2.5, 12: 4}
WO_PARTS = {9: (0,), 10: (1, 2), 11: (3,)}


def _comb(terms, get):
    v = get(terms[0][0])
    for i, sign in terms[1:]:
        a, b = v.astype(F32), get(i).astype(F32)
        v = a + b if sign > 0 else a - b
    return v


def _collector(emit):
    part = {}

    def push(j, val):
        for q, terms in enumerate(OUT):
            if j not in terms:
                continue
            if q not in part:
                part[q] = (val, terms[j], 1)
                continue
            v, sign, n = part[q]
            v = v + val if sign == terms[j] else v - val if sign > 0 else val - v
            part[q] = (v, 1, n + 1)
            if n + 1 == len(terms):
                emit(q, v)
    return push


def _block(q1, q2):
    return 2 * (q1 // 2) + q2 // 2, 2 * (q1 % 2) + q2 % 2


def _cols(c, n=128):
    return pl.ds(c * n, n)


def _ds(start, n):
    return pl.ds(start if isinstance(start, int) else pl.multiple_of(start, n), n)


def _dot(a, b):
    return jnp.dot(pltpu.bitcast(a, BF16), pltpu.bitcast(b, BF16), preferred_element_type=F32)


def _put7(table, quads, dst, pair, col, base=0):
    quads = [q.astype(F32) for q in quads]
    v = jnp.concatenate([_comb(terms, lambda q: quads[q]) for terms in table], axis=0).reshape(7, -1, 128)
    dst[pl.ds(base, 7), _ds(pair, v.shape[1] // 2), _cols(col)] = pltpu.bitcast(v.astype(BF16), U32)


def _put49(table, get, dst, pair, col, j):
    quads = [_comb(table[j], lambda q1: get(*_block(q1, q2))) for q2 in range(4)]
    _put7(table, quads, dst, pair, col, 7 * j)


def _weave(main, n, sides, lead):
    done = [0] * len(sides)
    for k in range(n):
        next(main)
        for s, side in enumerate(sides):
            upto = min(len(side), -(-len(side) * (k + 1) // (n - lead)))
            for job in side[done[s]:upto]:
                job()
            done[s] = upto


def _span(fn, size, unit, done, k):
    if k not in done:
        return []
    lo, hi = (int(round(done.get(i, 0) * size / unit)) * unit for i in (k - 1, k))
    jobs = []
    for t in range(NT):
        a, b = max(lo - t * size, 0), min(hi - t * size, size)
        jobs += fn(t, a, b) if a < b else []
    return jobs


def _start(copies):
    for c in copies:
        c.start()


def _wait(copies):
    for c in copies:
        c.wait()


def _kernel(x_hbm, wqkv_hbm, wo_hbm, wg_hbm, wu_hbm, wd_hbm, o_hbm,
            xb, wraw, wp0, wp1, wp2, tmpa, tmpb, tmpc, xa, qb, kb, vb, ha, ab, acc,
            rg, ru, rd, gu0, gu1, dn, sx, sw, sf, so, go):
    wp = (wp0, wp1, wp2, wp0)
    gu = (gu0, gu1)
    copy = pltpu.make_async_copy

    def block(fn):
        pl.when(go[0] > 0)(fn)

    def cp_x_half(t, i):
        return [copy(x_hbm.at[pl.ds(r, Q)], xb.at[pl.ds(r, Q)], sx.at[r // Q])
                for r in (t * TM + i * Q, t * TM + H + i * Q)]

    def cp_x(t):
        return [copy(x_hbm.at[pl.ds(t * TM, TM)], xb.at[pl.ds(t * TM, TM)], sx.at[6 + t])]

    def cp_wq(i):
        return [copy(wqkv_hbm.at[pl.ds(r, 128), pl.ds(0, D)], wraw.at[0, pl.ds(r, 128)], sw.at[r // 128])
                for r in (i * 128, D // 2 + i * 128)]

    def cp_w(m):
        return [copy(wqkv_hbm.at[:, pl.ds(m * D, D)] if m < 3 else wo_hbm, wraw.at[m % 2], sw.at[7 + m])]

    def cp_up(c, s):
        return [copy(src.at[:, _ds(c * FC, FC)], dst.at[s], sf.at[3 * s + i])
                for i, (src, dst) in enumerate(((wg_hbm, rg), (wu_hbm, ru)))]

    def cp_down(c, s):
        return [copy(wd_hbm.at[_ds(c * FC, FC)], rd.at[s], sf.at[3 * s + 2])]

    def layernorm(load, parts, finish, lo, hi, lag):
        mu, rs = {}, {}

        def mean(*rows):
            for r in rows:
                mu[r] = jnp.sum(load(r).sum(0), axis=-1, keepdims=True) * (1.0 / D)

        def rstd(*rows):
            for r in rows:
                xc = load(r) - mu[r]
                rs[r] = lax.rsqrt(jnp.sum((xc * xc).sum(0), axis=-1, keepdims=True) * (1.0 / D) + 1e-5)

        jobs = []
        for r in range(lo, hi + 2 * lag, 16):
            for fn, rr in ((mean, r), (rstd, r - lag)):
                if lo <= rr < hi:
                    jobs += [P(fn, rr + parts[i], rr + parts[i + 1]) for i in range(0, len(parts), 2)]
            if r - 2 * lag >= lo:
                jobs += finish(r - 2 * lag, lambda r, c: (load(r, c) - mu[r]) * rs[r])
        return jobs

    def ln1(t, lo, hi):
        def load(r, c=None):
            if c is None:
                return jnp.stack([load(r, c) for c in range(NCB)])
            return xb[pl.ds(t * TM + r, 16), _cols(c)].astype(F32)

        def put(r, c, norm):
            _put7(LHS, [norm(r + q // 2 * H, q % 2 * 4 + c) for q in range(4)], xa.at[t], r // 2, c)
        return layernorm(load, (0, H), lambda r, norm: [P(put, r, c, norm) for c in range(4)], lo, hi, 16)

    def ln2(t, lo, hi, lag=0):
        def load(r, c=slice(None)):
            return qb[c, pl.ds(t * TM + r, 16), :]

        def finish(r, norm):
            get = functools.cache(lambda c, i, k: norm(r + i * Q, 2 * k + c))
            return [P(_put49, LHS, P(get, c), ha.at[t], r // 2, c, j) for c in range(2) for j in range(7)]
        return layernorm(load, (0, Q, 2 * Q, 3 * Q), finish, lo, hi, lag)

    def prep_cols(m, i):
        tmp = (tmpa, tmpb)[i % 2]

        def fwd(c):
            w = jnp.concatenate([wraw[m % 2, pl.ds(b + i * 128, 128), _cols(c)] for b in (0, D // 2)], axis=0)
            wt = pltpu.bitcast(w, U32).T
            for h in range(4):
                tmp[pl.ds((4 * c + h) * PITCH, DH), :] = wt[h * DH:(h + 1) * DH]

        def back(c):
            rows = [tmp[pl.ds(4 * c + d, NH, stride=PITCH), :] for d in range(4)]
            tmpc[_cols(c), :] = jnp.concatenate(rows, axis=0).T

        def put(c, r0):
            for r in range(r0, r0 + 32, 8):
                quads = [tmpc[pl.ds((q % 2 * 4 + c) * 128 + q // 2 * 64 + r, 8), :] for q in range(4)]
                _put7(RHS, [pltpu.bitcast(v, BF16) for v in quads], wp[m], i * 64 + r, c)
        return ([P(fwd, c) for c in range(NCB)] + [P(back, c) for c in (0, 4, 1, 5, 2, 6, 3, 7)]
                + [P(put, c, r) for c in range(4) for r in (0, 32)])

    def prep_rows(i):
        def fwd(n, h0):
            for h in (h0, h0 + 1):
                w = wraw[1, pl.ds(h * DH, DH), _cols(4 * n + i)].astype(F32)
                (tmpa, tmpb)[n][pl.ds(h * PITCH, DH), :] = pltpu.bitcast(w, U32)

        def put(d):
            for h in (0, 16):
                quads = [(tmpa, tmpb)[q % 2][pl.ds(h * PITCH + q // 2 * 16 + d, 16, stride=PITCH), :]
                         for q in range(4)]
                _put7(RHS, [pltpu.bitcast(v, F32) for v in quads], wp[3], d * 16 + h // 2, i)
        return [P(fwd, n, h) for n in range(2) for h in range(0, NH, 2)] + [P(put, d) for d in range(16)]

    def prep_ffn(src, s, t, rows, cols, c, dst, pair, col):
        def get(r, k, n):
            return src[s, _ds(k * rows + t * (rows // NT) + r, 16), pl.ds(n * cols + c * 128, 128)]
        return [P(_put49, RHS, P(get, r), dst, pair + t * (rows // NT // 2) + r // 2, col, j)
                for r in range(0, rows // NT, 16) for j in range(7)]

    def prep_up(s, t):
        return sum((prep_ffn(src, s, t, D // 4, FC // 4, 0, gu[s], 0, i) for i, src in enumerate((rg, ru))), [])

    def prep_down(s, t):
        return sum((prep_ffn(rd, s, t, FC // 4, D // 4, c, dn, s * FC // 8, c) for c in range(2)), [])

    def probs(t, lo, hi):
        st = {}

        def dots(r, w):
            k = kb[:, pl.ds(t * TM + r + HALO - DIL * w, 8), :]
            for rr, ww in ((r, w), (r + 8, w + 8 // DIL)):
                if lo <= rr < hi:
                    st[rr, ww] = (qb[:, pl.ds(t * TM + rr, 8), :] * k).sum(0)

        def fold(r):
            l = jnp.concatenate([st[r, w] for w in range(WIN)], axis=0)
            st[r] = l + pltpu.roll(l, 64, 1)

        def softmax(r):
            l = (st[r] + pltpu.roll(st[r], 32, 1)) * (DH ** -0.5 * LOG2E)
            l = l.reshape(WIN, 8, 128)
            if t * TM + r < DIL * (WIN - 1):
                pos = t * TM + r + lax.broadcasted_iota(jnp.int32, l.shape, 1)
                l = jnp.where(pos >= DIL * lax.broadcasted_iota(jnp.int32, l.shape, 0), l, -1e9 * LOG2E)
            p = jnp.exp2(l - l.max(0))
            qb[:, pl.ds(t * TM + r, 8), :] = p * (1.0 / p.sum(0))

        jobs = [P(dots, lo - 8, w) for w in range(4)]
        for r in range(lo, hi, 8):
            jobs += [P(dots, r, w) for w in range(4)] + [P(fold, r)] + ([P(softmax, r - 8)] if r > lo else [])
        return jobs + [P(softmax, hi - 8)]

    def mix(t, lo, hi):
        st = {}

        def part(r, c, i):
            r0 = t * TM + i * H + r
            for w in range(WIN):
                pv = qb[w, pl.ds(r0, 16), :] * vb[pl.ds(2 * c, 2), pl.ds(r0 + HALO - DIL * w, 16), :]
                st[i] = st[i] + pv if w else pv
            if i:
                _put7(LHS, [st[q // 2][q % 2] for q in range(4)], xa.at[t], r // 2, c)
        return [P(part, r, c, i) for r in range(lo, hi, 16) for c in range(4) for i in range(2)]

    head, tail = prep_cols(0, 0), ln1(0, Q, H)
    for n, job in enumerate(head[2 * NCB:]):
        tail.insert(7 * n, job)
    go[0] = 1
    _start(cp_x_half(0, 0) + cp_wq(0))
    kb[:, pl.ds(0, HALO), :] = jnp.zeros((NCB, HALO, 128), F32)
    for now, later, jobs in ((cp_x_half(0, 0), cp_x_half(0, 1), ln1(0, 0, Q)),
                             (cp_wq(0), cp_wq(1), head[:2 * NCB]),
                             (cp_x_half(0, 1), cp_wq(2), tail)):
        _wait(now)
        _start(later)
        for job in jobs:
            job()

    def boot(i):
        if i == 0:
            _start(cp_wq(3))
            sides = [[lambda: None] * 6 + [lambda: _wait(cp_wq(1))] + prep_cols(0, 1)]
        elif i == 1:
            _wait(cp_wq(2))
            _start(cp_x_half(1, 0))
            sides = [prep_cols(0, 2)]
        elif i == 2:
            _wait(cp_wq(3) + cp_x_half(1, 0))
            _start(cp_x_half(1, 1))
            sides = [prep_cols(0, 3), ln1(1, 0, 48)]
        else:
            _start(cp_w(1))
            sides = [ln1(1, 48, Q)]

        def stages():
            for r in range(2):
                for n in range(2):
                    def emit(q, val):
                        for c in range(2):
                            qb[q % 2 * 4 + 2 * n + c, pl.ds(q // 2 * H + r * Q, Q), :] = val[:, c * 128:(c + 1) * 128]
                    push = _collector(emit)
                    for j in PROJ_ORDER:
                        val = _dot(xa[0, j, _cols(r, Q // 2), _cols(i)], wp0[j, _cols(i, 64), _cols(n, 256)])
                        val = val + acc[2 * r + n, j] if i else val
                        if i < 3:
                            acc[2 * r + n, j] = val
                        else:
                            push(j, val)
                        yield
        _weave(stages(), 28, sides, 2)

    def step(k):
        m, t, rows, lo, hi = STEPS[k]
        prep = sum((prep_rows(i) for i in WO_PARTS.get(k, ())), [])
        if k == 0:
            _wait(cp_x_half(1, 1))
            _start(cp_x(2))
        elif k == 1:
            _wait(cp_w(1))
            _start(cp_x(3))
            prep = sum((prep_cols(1, i) for i in range(4)), [])
        elif k == 2:
            _wait(cp_x(2) + cp_x(3))
            _start(cp_w(2) + cp_up(0, 0) + cp_down(0, 0))
        elif k == 3:
            _start(cp_w(3))
        elif k == 4:
            _wait(cp_w(2))
            _start(cp_up(1, 1))
        elif k == 7:
            _wait(cp_w(3) + cp_up(0, 0) + cp_down(0, 0) + cp_up(1, 1))
        elif k == 9:
            vb[:, pl.ds(0, HALO), :] = jnp.broadcast_to(vb[:, pl.ds(HALO, 1), :], (NCB, HALO, 128))
        if 4 <= k < 8:
            prep = prep_cols(2, k - 4)
        sides = [_span(ln1, H, 16, LN1_DONE, k), _span(probs, TM, 8, PROBS_DONE, k), _span(mix, H, 16, MIX_DONE, k),
                 prep, _span(lambda t, a, b: (prep_up(0, t) + prep_down(0, t))[a:b], 84, 1, FFN0_DONE, k), _span(ln2, Q, 16, LN2_DONE, k),
                 prep_up(1, 0) if k == 11 else []]

        def stages():
            for n in range(4):
                for r in range(lo, hi, rows):
                    def emit(q, val):
                        r0, c = t * TM + q // 2 * H + r, q % 2 * 4 + n
                        if m == 0:
                            qb[c, pl.ds(r0, rows), :] = val
                        elif m == 1:
                            kb[c, pl.ds(HALO + r0, rows), :] = val
                        elif m == 2:
                            vb[2 * n + q % 2, pl.ds(HALO + r0, rows), :] = val
                        else:
                            qb[c, pl.ds(r0, rows), :] = val + xb[pl.ds(r0, rows), _cols(c)].astype(F32)
                    push = _collector(emit)
                    for j in PROJ_ORDER:
                        push(j, _dot(xa[t, j, pl.ds(r // 2, rows // 2), :], wp[m][j, :, _cols(n)]))
                        yield
        _weave(stages(), 28 * ((hi - lo) // rows), sides, (hi - lo) // rows)

    for i in range(4):
        block(P(boot, i))
    for k in range(len(STEPS)):
        block(P(step, k))

    def ffn(s, t, side, first=False, last=False):
        act = {}

        def parked(i, n):
            return n, _ds(t * TM + i * Q, Q), slice(None)

        def geglu(q2, q1, val):
            g, u = val[:, :128], val[:, 128:]
            a = (g * u) * (jnp.tanh(g * (g * g * G1 + G0)) * 0.5 + 0.5)
            if s:
                kb[parked(*_block(q1, q2))] = a
            else:
                act[_block(q1, q2)] = a

        def store(q2, q1, val):
            i, n = _block(q1, q2)
            rows = _ds(t * TM + i * Q, Q)
            for c in range(2):
                xb[rows, _cols(2 * n + c)] = (qb[2 * n + c, rows, :] + val[:, c * 128:(c + 1) * 128]).astype(BF16)
            copy(xb.at[rows, _cols(n, 256)], o_hbm.at[rows, _cols(n, 256)], so).start()

        def down(j):
            if first:
                return _dot(ab[j, :, _cols(0)], dn[j, _cols(0, FC // 8), :])
            return acc[t, j] + _dot(ab[j], dn[j])

        def combine(j1, outer, order, product):
            inner = _collector(lambda q2, v: outer[q2](j1, v))
            for j2 in order:
                inner(j2, product(7 * j1 + j2))
                yield

        def accumulate(j1):
            for j in range(7 * j1, 7 * j1 + 7):
                acc[t, j] = down(j)
                yield

        def stages():
            ups, downs = FFN_PLAN_LAST if last else FFN_PLAN
            up = [_collector(P(geglu, q2)) for q2 in range(4)]
            out = [_collector(P(store, q2)) for q2 in range(4)]
            groups = [combine(j1, up, UP_ORDER, lambda j: _dot(ha[t, j], gu[s][j])) for j1 in ups]
            groups += [combine(j1, out, DOWN_ORDER, down) if last else accumulate(j1) for j1 in downs]
            for n, group in enumerate(groups):
                yield from group
                if 4 <= n < 11 and not s:
                    _put49(LHS, lambda i, k: act[i, k], ab, 0, 0, downs[n - 4])
                if n in PARKED and not (s or first):
                    for j in PARKED[n]:
                        _put49(LHS, lambda i, k: kb[parked(i, k)], ab, 0, 1, downs[j])
        _weave(stages(), 49 if s else 98, [side], 3)

    def fetch(c):
        return cp_up(c + 1, 0) + cp_down(c, 1) + cp_down(c + 1, 0)

    def enter():
        _start(fetch(1))
        ffn(0, 0, ln2(NT - 1, 0, Q, 16), first=True)

    def pair(p, _):
        c, more = 2 * p + 1, p < NF // 2 - 1
        _wait(fetch(c))
        pl.when(more)(lambda: _start(cp_up(c + 2, 1)))
        lax.fori_loop(0, NT, lambda t, _: ffn(1, t, prep_up(0, t) + prep_down(0, t) + prep_down(1, t)), None)

        @pl.when(more)
        def _():
            _wait(cp_up(c + 2, 1))
            _start(fetch(c + 2))
            lax.fori_loop(0, NT, lambda t, _: ffn(0, t, prep_up(1, t)), None)

    block(enter)
    lax.fori_loop(1, NT, lambda t, _: ffn(0, t, prep_up(1, t), first=True), None)
    lax.fori_loop(0, NF // 2, pair, None)
    lax.fori_loop(0, NT, lambda t, _: ffn(0, t, [], last=True), None)
    copy(xb, o_hbm, so).wait()


@jax.jit
def pallas_sequential_preLN__sliding_local_dilated__glu_gated_geglu__prompt_kernel(
    A_x: jax.Array,
    A_wqkv: jax.Array,
    A_wo: jax.Array,
    B_x: jax.Array,
    B_w_gate: jax.Array,
    B_w_up: jax.Array,
    B_w_down: jax.Array,
):
    del B_x
    hbm = pl.BlockSpec(memory_space=pl.ANY)
    vmem, dma = pltpu.VMEM, pltpu.SemaphoreType.DMA
    out = pl.pallas_call(
        _kernel,
        in_specs=[hbm] * 6,
        out_specs=hbm,
        out_shape=jax.ShapeDtypeStruct((S, D), BF16),
        scratch_shapes=(
            [vmem((S, D), BF16), vmem((2, D, D), BF16)] + [vmem((7, D // 4, D // 2), U32)] * 3
            + [vmem((NH * PITCH + DH, 128), U32)] * 2 + [vmem((D, 128), U32), vmem((NT, 7, H // 2, D // 2), U32)]
            + [vmem((NCB, S, 128), F32)] + [vmem((NCB, HALO + S, 128), F32)] * 2
            + [vmem((NT, 49, Q // 2, D // 4), U32), vmem((49, Q // 2, FC // 2), U32), vmem((NT, 49, Q, D // 4), F32)]
            + [vmem((2, D, FC), BF16), vmem((2, D, FC), BF16), vmem((2, FC, D), BF16)]
            + [vmem((49, D // 8, FC // 2), U32)] * 2 + [vmem((49, FC // 4, D // 4), U32)]
            + [dma((10,)), dma((11,)), dma((6,)), dma(()), pltpu.SMEM((1,), jnp.int32)]),
        compiler_params=pltpu.CompilerParams(
            vmem_limit_bytes=122 * 2 ** 20,
            flags={"XLA_TPU_EVENLY_DISTRIBUTE_CRITICAL_NODES": True},
        ),
    )(A_x.reshape(S, D), A_wqkv, A_wo, B_w_gate, B_w_up, B_w_down)
    return out.reshape(1, S, D)
```

```python
import functools

import jax
import jax.experimental.pallas as pl
import jax.experimental.pallas.tpu as pltpu
import jax.numpy as jnp
import numpy as np
from jax import lax

S, D, F = 2048, 1024, 3584
NH, DH, WIN, DIL = 32, 32, 8, 2
TM, FC = 512, 512
NT, NF = S // TM, F // FC
H, Q = TM // 2, TM // 4
NCB = D // 128
HALO = 16
PITCH = DH + 1
F32, BF16, U32 = jnp.float32, jnp.bfloat16, jnp.uint32
LOG2E = float(np.log2(np.e))
G0 = float(np.sqrt(2.0 / np.pi))
G1 = G0 * 0.044715
P = functools.partial

LHS = (((0, 1), (3, 1)), ((2, 1), (3, 1)), ((0, 1),), ((3, 1),), ((0, 1), (1, 1)), ((2, 1), (0, -1)), ((1, 1), (3, -1)))
RHS = (((0, 1), (3, 1)), ((0, 1),), ((1, 1), (3, -1)), ((2, 1), (0, -1)), ((3, 1),), ((0, 1), (1, 1)), ((2, 1), (3, 1)))
OUT = ({0: 1, 3: 1, 4: -1, 6: 1}, {2: 1, 4: 1}, {1: 1, 3: 1}, {0: 1, 1: -1, 2: 1, 5: 1})

ORDER = (1, 3, 2, 4, 0, 5, 6)
FFN_PLAN = ((0, 4, 6, 3, 1, 2, 5), (2, 5, 4, 3, 1, 6, 0))
FFN_PLAN_ODD = ((1, 3, 2, 4, 0, 5, 6), ())
FFN_PLAN_LAST = ((0, 1, 2, 5, 4, 3, 6), (3, 6, 1, 0, 4, 2, 5))

STEPS = ((0, 1, Q, 0, Q), (0, 1, Q, Q, H), (1, 0, H, 0, H), (1, 1, H, 0, H),
         (0, 2, H, 0, H), (1, 2, H, 0, H), (0, 3, H, 0, H), (1, 3, H, 0, H),
         (2, 0, H, 0, H), (2, 1, 64, 0, H), (2, 2, 64, 0, H), (2, 3, 64, 0, H),
         (3, 0, 64, 0, H), (3, 1, H, 0, H), (3, 2, H, 0, H), (3, 3, H, 0, H))
LN1_DONE = {-1: 1.5, 0: 2, 1: 2, 2: 3.25, 3: 3.5, 4: 3.75, 5: 4}
PROBS_DONE = {3: 0.6875, 4: 1.25, 5: 1.8125, 6: 2.4375, 7: 3, 8: 4}
MIX_DONE = {9: 1, 10: 2, 11: 3, 12: 4}
LN2_DONE = {13: 1, 14: 2, 15: 3}
FFN0_DONE = {9: 1, 10: 1.5, 11: 2.5, 12: 4}
WO_PARTS = {9: (0,), 10: (1, 2), 11: (3,)}


def _comb(terms, get):
    v = get(terms[0][0])
    for i, sign in terms[1:]:
        a, b = v.astype(F32), get(i).astype(F32)
        v = a + b if sign > 0 else a - b
    return v


def _collector(emit):
    part = {}

    def push(j, val):
        for q, terms in enumerate(OUT):
            if j not in terms:
                continue
            if q not in part:
                part[q] = (val, terms[j], 1)
                continue
            v, sign, n = part[q]
            v = v + val if sign == terms[j] else v - val if sign > 0 else val - v
            part[q] = (v, 1, n + 1)
            if n + 1 == len(terms):
                emit(q, v)
    return push


def _block(q1, q2):
    return 2 * (q1 // 2) + q2 // 2, 2 * (q1 % 2) + q2 % 2


def _cols(c, n=128):
    return pl.ds(c * n, n)


def _ds(start, n):
    return pl.ds(start if isinstance(start, int) else pl.multiple_of(start, n), n)


def _dot(a, b):
    return jnp.dot(pltpu.bitcast(a, BF16), pltpu.bitcast(b, BF16), preferred_element_type=F32)


def _put7(table, quads, dst, pair, col, base=0):
    quads = [q.astype(F32) for q in quads]
    v = jnp.concatenate([_comb(terms, lambda q: quads[q]) for terms in table], axis=0).reshape(7, -1, 128)
    dst[pl.ds(base, 7), _ds(pair, v.shape[1] // 2), _cols(col)] = pltpu.bitcast(v.astype(BF16), U32)


def _put49(table, get, dst, pair, col, j):
    quads = [_comb(table[j], lambda q1: get(*_block(q1, q2))) for q2 in range(4)]
    _put7(table, quads, dst, pair, col, 7 * j)


def _weave(main, n, sides, lead):
    done = [0] * len(sides)
    for k in range(n):
        next(main)
        for s, side in enumerate(sides):
            upto = min(len(side), -(-len(side) * (k + 1) // (n - lead)))
            for job in side[done[s]:upto]:
                job()
            done[s] = upto


def _span(fn, size, unit, done, k):
    if k not in done:
        return []
    lo, hi = (int(round(done.get(i, 0) * size / unit)) * unit for i in (k - 1, k))
    jobs = []
    for t in range(NT):
        a, b = max(lo - t * size, 0), min(hi - t * size, size)
        jobs += fn(t, a, b) if a < b else []
    return jobs


def _start(copies):
    for c in copies:
        c.start()


def _wait(copies):
    for c in copies:
        c.wait()


def _kernel(x_hbm, wqkv_hbm, wo_hbm, wg_hbm, wu_hbm, wd_hbm, o_hbm,
            xb, wraw, wp0, wp1, wp2, tmpa, tmpb, tmpc, xa, qb, kb, vb, ha, ab, acc,
            rg, ru, rd, gu0, gu1, dn, sx, sw, sf, so, go):
    wp = (wp0, wp1, wp2, wp0)
    gu = (gu0, gu1)
    copy = pltpu.make_async_copy

    def block(fn):
        pl.when(go[0] > 0)(fn)

    def cp_x_half(t, i):
        return [copy(x_hbm.at[pl.ds(r, Q)], xb.at[pl.ds(r, Q)], sx.at[r // Q])
                for r in (t * TM + i * Q, t * TM + H + i * Q)]

    def cp_x(t):
        return [copy(x_hbm.at[pl.ds(t * TM, TM)], xb.at[pl.ds(t * TM, TM)], sx.at[6 + t])]

    def cp_wq(i):
        return [copy(wqkv_hbm.at[pl.ds(r, 128), pl.ds(0, D)], wraw.at[0, pl.ds(r, 128)], sw.at[r // 128])
                for r in (i * 128, D // 2 + i * 128)]

    def cp_w(m):
        return [copy(wqkv_hbm.at[:, pl.ds(m * D, D)] if m < 3 else wo_hbm, wraw.at[m % 2], sw.at[7 + m])]

    def cp_up(c, s):
        return [copy(src.at[:, _ds(c * FC, FC)], dst.at[s], sf.at[3 * s + i])
                for i, (src, dst) in enumerate(((wg_hbm, rg), (wu_hbm, ru)))]

    def cp_down(c, s):
        return [copy(wd_hbm.at[_ds(c * FC, FC)], rd.at[s], sf.at[3 * s + 2])]

    def layernorm(load, parts, finish, lo, hi, lag):
        mu, rs = {}, {}

        def mean(*rows):
            for r in rows:
                mu[r] = jnp.sum(load(r).sum(0), axis=-1, keepdims=True) * (1.0 / D)

        def rstd(*rows):
            for r in rows:
                xc = load(r) - mu[r]
                rs[r] = lax.rsqrt(jnp.sum((xc * xc).sum(0), axis=-1, keepdims=True) * (1.0 / D) + 1e-5)

        jobs = []
        for r in range(lo, hi + 2 * lag, 16):
            for fn, rr in ((mean, r), (rstd, r - lag)):
                if lo <= rr < hi:
                    jobs += [P(fn, rr + parts[i], rr + parts[i + 1]) for i in range(0, len(parts), 2)]
            if r - 2 * lag >= lo:
                jobs += finish(r - 2 * lag, lambda r, c: (load(r, c) - mu[r]) * rs[r])
        return jobs

    def ln1(t, lo, hi):
        def load(r, c=None):
            if c is None:
                return jnp.stack([load(r, c) for c in range(NCB)])
            return xb[pl.ds(t * TM + r, 16), _cols(c)].astype(F32)

        def put(r, c, norm):
            _put7(LHS, [norm(r + q // 2 * H, q % 2 * 4 + c) for q in range(4)], xa.at[t], r // 2, c)
        return layernorm(load, (0, H), lambda r, norm: [P(put, r, c, norm) for c in range(4)], lo, hi, 16)

    def ln2(t, lo, hi, lag=0):
        def load(r, c=slice(None)):
            return qb[c, pl.ds(t * TM + r, 16), :]

        def finish(r, norm):
            get = functools.cache(lambda c, i, k: norm(r + i * Q, 2 * k + c))
            return [P(_put49, LHS, P(get, c), ha.at[t], r // 2, c, j) for c in range(2) for j in range(7)]
        return layernorm(load, (0, Q, 2 * Q, 3 * Q), finish, lo, hi, lag)

    def prep_cols(m, i):
        tmp = (tmpa, tmpb)[i % 2]

        def fwd(c):
            w = jnp.concatenate([wraw[m % 2, pl.ds(b + i * 128, 128), _cols(c)] for b in (0, D // 2)], axis=0)
            wt = pltpu.bitcast(w, U32).T
            for h in range(4):
                tmp[pl.ds((4 * c + h) * PITCH, DH), :] = wt[h * DH:(h + 1) * DH]

        def back(c):
            rows = [tmp[pl.ds(4 * c + d, NH, stride=PITCH), :] for d in range(4)]
            tmpc[_cols(c), :] = jnp.concatenate(rows, axis=0).T

        def put(c, r0):
            for r in range(r0, r0 + 32, 8):
                quads = [tmpc[pl.ds((q % 2 * 4 + c) * 128 + q // 2 * 64 + r, 8), :] for q in range(4)]
                _put7(RHS, [pltpu.bitcast(v, BF16) for v in quads], wp[m], i * 64 + r, c)
        return ([P(fwd, c) for c in range(NCB)] + [P(back, c) for c in (0, 4, 1, 5, 2, 6, 3, 7)]
                + [P(put, c, r) for c in range(4) for r in (0, 32)])

    def prep_rows(i):
        def fwd(n, h0):
            for h in (h0, h0 + 1):
                w = wraw[1, pl.ds(h * DH, DH), _cols(4 * n + i)].astype(F32)
                (tmpa, tmpb)[n][pl.ds(h * PITCH, DH), :] = pltpu.bitcast(w, U32)

        def put(d):
            for h in (0, 16):
                quads = [(tmpa, tmpb)[q % 2][pl.ds(h * PITCH + q // 2 * 16 + d, 16, stride=PITCH), :]
                         for q in range(4)]
                _put7(RHS, [pltpu.bitcast(v, F32) for v in quads], wp[3], d * 16 + h // 2, i)
        return [P(fwd, n, h) for n in range(2) for h in range(0, NH, 2)] + [P(put, d) for d in range(16)]

    def prep_ffn(src, s, t, rows, cols, c, dst, pair, col):
        def get(r, k, n):
            return src[s, _ds(k * rows + t * (rows // NT) + r, 16), pl.ds(n * cols + c * 128, 128)]
        return [P(_put49, RHS, P(get, r), dst, pair + t * (rows // NT // 2) + r // 2, col, j)
                for r in range(0, rows // NT, 16) for j in range(7)]

    def prep_up(s, t):
        return sum((prep_ffn(src, s, t, D // 4, FC // 4, 0, gu[s], 0, i) for i, src in enumerate((rg, ru))), [])

    def prep_down(s, t):
        return sum((prep_ffn(rd, s, t, FC // 4, D // 4, c, dn, s * FC // 8, c) for c in range(2)), [])

    def probs(t, lo, hi):
        st = {}

        def dots(r, w):
            k = kb[:, pl.ds(t * TM + r + HALO - DIL * w, 8), :]
            for rr, ww in ((r, w), (r + 8, w + 8 // DIL)):
                if lo <= rr < hi:
                    st[rr, ww] = (qb[:, pl.ds(t * TM + rr, 8), :] * k).sum(0)

        def fold(r):
            l = jnp.concatenate([st[r, w] for w in range(WIN)], axis=0)
            st[r] = l + pltpu.roll(l, 64, 1)

        def softmax(r):
            l = (st[r] + pltpu.roll(st[r], 32, 1)) * (DH ** -0.5 * LOG2E)
            l = l.reshape(WIN, 8, 128)
            if t * TM + r < DIL * (WIN - 1):
                pos = t * TM + r + lax.broadcasted_iota(jnp.int32, l.shape, 1)
                l = jnp.where(pos >= DIL * lax.broadcasted_iota(jnp.int32, l.shape, 0), l, -1e9 * LOG2E)
            p = jnp.exp2(l - l.max(0))
            qb[:, pl.ds(t * TM + r, 8), :] = p * (1.0 / p.sum(0))

        jobs = [P(dots, lo - 8, w) for w in range(4)]
        for r in range(lo, hi, 8):
            jobs += [P(dots, r, w) for w in range(4)] + [P(fold, r)] + ([P(softmax, r - 8)] if r > lo else [])
        return jobs + [P(softmax, hi - 8)]

    def mix(t, lo, hi):
        st = {}

        def part(r, c, i):
            r0 = t * TM + i * H + r
            for w in range(WIN):
                pv = qb[w, pl.ds(r0, 16), :] * vb[pl.ds(2 * c, 2), pl.ds(r0 + HALO - DIL * w, 16), :]
                st[i] = st[i] + pv if w else pv
            if i:
                _put7(LHS, [st[q // 2][q % 2] for q in range(4)], xa.at[t], r // 2, c)
        return [P(part, r, c, i) for r in range(lo, hi, 16) for c in range(4) for i in range(2)]

    head, tail = prep_cols(0, 0), ln1(0, Q, H)
    for n, job in enumerate(head[2 * NCB:]):
        tail.insert(7 * n, job)
    go[0] = 1
    _start(cp_x_half(0, 0) + cp_wq(0))
    kb[:, pl.ds(0, HALO), :] = jnp.zeros((NCB, HALO, 128), F32)
    for now, later, jobs in ((cp_x_half(0, 0), cp_x_half(0, 1), ln1(0, 0, Q)),
                             (cp_wq(0), cp_wq(1), head[:2 * NCB]),
                             (cp_x_half(0, 1), cp_wq(2), tail)):
        _wait(now)
        _start(later)
        for job in jobs:
            job()

    def boot(i):
        if i == 0:
            _start(cp_wq(3))
            sides = [[lambda: None] * 6 + [lambda: _wait(cp_wq(1))] + prep_cols(0, 1)]
        elif i == 1:
            _wait(cp_wq(2))
            _start(cp_x_half(1, 0))
            sides = [prep_cols(0, 2)]
        elif i == 2:
            _wait(cp_wq(3) + cp_x_half(1, 0))
            _start(cp_x_half(1, 1))
            sides = [prep_cols(0, 3), ln1(1, 0, 48)]
        else:
            _start(cp_w(1))
            sides = [ln1(1, 48, Q)]

        def stages():
            for r in range(2):
                for n in range(2):
                    def emit(q, val):
                        for c in range(2):
                            qb[q % 2 * 4 + 2 * n + c, pl.ds(q // 2 * H + r * Q, Q), :] = val[:, c * 128:(c + 1) * 128]
                    push = _collector(emit)
                    for j in ORDER:
                        val = _dot(xa[0, j, _cols(r, Q // 2), _cols(i)], wp0[j, _cols(i, 64), _cols(n, 256)])
                        val = val + acc[2 * r + n, j] if i else val
                        if i < 3:
                            acc[2 * r + n, j] = val
                        else:
                            push(j, val)
                        yield
        _weave(stages(), 28, sides, 2)

    def step(k):
        m, t, rows, lo, hi = STEPS[k]
        prep = sum((prep_rows(i) for i in WO_PARTS.get(k, ())), [])
        if k == 0:
            _wait(cp_x_half(1, 1))
            _start(cp_x(2))
        elif k == 1:
            _wait(cp_w(1))
            _start(cp_x(3))
            prep = sum((prep_cols(1, i) for i in range(4)), [])
        elif k == 2:
            _wait(cp_x(2) + cp_x(3))
            _start(cp_w(2) + cp_up(0, 0) + cp_down(0, 0))
        elif k == 3:
            _start(cp_w(3))
        elif k == 4:
            _wait(cp_w(2))
            _start(cp_up(1, 1))
        elif k == 7:
            _wait(cp_w(3) + cp_up(0, 0) + cp_down(0, 0) + cp_up(1, 1))
        elif k == 9:
            vb[:, pl.ds(0, HALO), :] = jnp.broadcast_to(vb[:, pl.ds(HALO, 1), :], (NCB, HALO, 128))
        if 4 <= k < 8:
            prep = prep_cols(2, k - 4)
        sides = [_span(ln1, H, 16, LN1_DONE, k), _span(probs, TM, 8, PROBS_DONE, k), _span(mix, H, 16, MIX_DONE, k),
                 prep, _span(lambda t, a, b: (prep_up(0, t) + prep_down(0, t))[a:b], 84, 1, FFN0_DONE, k), _span(ln2, Q, 16, LN2_DONE, k),
                 prep_up(1, 0) if k == 11 else []]

        def stages():
            for n in range(4):
                for r in range(lo, hi, rows):
                    def emit(q, val):
                        r0, c = t * TM + q // 2 * H + r, q % 2 * 4 + n
                        if m == 0:
                            qb[c, pl.ds(r0, rows), :] = val
                        elif m == 1:
                            kb[c, pl.ds(HALO + r0, rows), :] = val
                        elif m == 2:
                            vb[2 * n + q % 2, pl.ds(HALO + r0, rows), :] = val
                        else:
                            qb[c, pl.ds(r0, rows), :] = val + xb[pl.ds(r0, rows), _cols(c)].astype(F32)
                    push = _collector(emit)
                    for j in ORDER:
                        push(j, _dot(xa[t, j, pl.ds(r // 2, rows // 2), :], wp[m][j, :, _cols(n)]))
                        yield
        _weave(stages(), 28 * ((hi - lo) // rows), sides, (hi - lo) // rows)

    for i in range(4):
        block(P(boot, i))
    for k in range(len(STEPS)):
        block(P(step, k))

    def ffn(s, t, side, first=False, last=False):
        act = {}

        def parked(i, n):
            return n, _ds(t * TM + i * Q, Q), slice(None)

        def geglu(q2, q1, val):
            g, u = val[:, :128], val[:, 128:]
            a = (g * u) * (jnp.tanh(g * (g * g * G1 + G0)) * 0.5 + 0.5)
            if s:
                kb[parked(*_block(q1, q2))] = a
            else:
                act[_block(q1, q2)] = a

        def store(q2, q1, val):
            i, n = _block(q1, q2)
            rows = _ds(t * TM + i * Q, Q)
            for c in range(2):
                xb[rows, _cols(2 * n + c)] = (qb[2 * n + c, rows, :] + val[:, c * 128:(c + 1) * 128]).astype(BF16)
            copy(xb.at[rows, _cols(n, 256)], o_hbm.at[rows, _cols(n, 256)], so).start()

        def down(j):
            if first:
                return _dot(ab[j, :, _cols(0)], dn[j, _cols(0, FC // 8), :])
            return acc[t, j] + _dot(ab[j], dn[j])

        def combine(j1, outer, product):
            inner = _collector(lambda q2, v: outer[q2](j1, v))
            for j2 in ORDER:
                inner(j2, product(7 * j1 + j2))
                yield

        def accumulate(j1):
            for j in range(7 * j1, 7 * j1 + 7):
                acc[t, j] = down(j)
                yield

        def stages():
            ups, downs = FFN_PLAN_LAST if last else FFN_PLAN_ODD if s else FFN_PLAN
            up = [_collector(P(geglu, q2)) for q2 in range(4)]
            out = [_collector(P(store, q2)) for q2 in range(4)]
            groups = [combine(j1, up, lambda j: _dot(ha[t, j], gu[s][j])) for j1 in ups]
            groups += [combine(j1, out, down) if last else accumulate(j1) for j1 in downs]
            for n, group in enumerate(groups):
                yield from group
                if 4 <= n < 11 and not s:
                    _put49(LHS, lambda i, k: act[i, k], ab, 0, 0, downs[n - 4])
                    if not first:
                        _put49(LHS, lambda i, k: kb[parked(i, k)], ab, 0, 1, downs[n - 4])
        _weave(stages(), 49 if s else 98, [side], 3)

    def tiles(fn, unroll=1):
        def body(i, _):
            for u in range(unroll):
                fn(i * unroll + u)
        lax.fori_loop(0, NT // unroll, body, None)

    def fetch(c):
        return cp_up(c + 1, 0) + cp_down(c, 1) + cp_down(c + 1, 0)

    def enter():
        _start(fetch(1))
        ffn(0, 0, ln2(NT - 1, 0, Q, 16), first=True)

    def pair(p, _):
        c, more = 2 * p + 1, p < NF // 2 - 1
        _wait(fetch(c))
        pl.when(more)(lambda: _start(cp_up(c + 2, 1)))
        tiles(lambda t: ffn(1, t, prep_up(0, t) + prep_down(0, t) + prep_down(1, t)), 2)

        @pl.when(more)
        def _():
            _wait(cp_up(c + 2, 1))
            _start(fetch(c + 2))
            tiles(lambda t: ffn(0, t, prep_up(1, t)))

    block(enter)
    lax.fori_loop(1, NT, lambda t, _: ffn(0, t, prep_up(1, t), first=True), None)
    lax.fori_loop(0, NF // 2, pair, None)
    tiles(lambda t: ffn(0, t, [], last=True))
    copy(xb, o_hbm, so).wait()


@jax.jit
def pallas_sequential_preLN__sliding_local_dilated__glu_gated_geglu__prompt_kernel(
    A_x: jax.Array,
    A_wqkv: jax.Array,
    A_wo: jax.Array,
    B_x: jax.Array,
    B_w_gate: jax.Array,
    B_w_up: jax.Array,
    B_w_down: jax.Array,
):
    del B_x
    hbm = pl.BlockSpec(memory_space=pl.ANY)
    vmem, dma = pltpu.VMEM, pltpu.SemaphoreType.DMA
    out = pl.pallas_call(
        _kernel,
        in_specs=[hbm] * 6,
        out_specs=hbm,
        out_shape=jax.ShapeDtypeStruct((S, D), BF16),
        scratch_shapes=(
            [vmem((S, D), BF16), vmem((2, D, D), BF16)] + [vmem((7, D // 4, D // 2), U32)] * 3
            + [vmem((NH * PITCH + DH, 128), U32)] * 2 + [vmem((D, 128), U32), vmem((NT, 7, H // 2, D // 2), U32)]
            + [vmem((NCB, S, 128), F32)] + [vmem((NCB, HALO + S, 128), F32)] * 2
            + [vmem((NT, 49, Q // 2, D // 4), U32), vmem((49, Q // 2, FC // 2), U32), vmem((NT, 49, Q, D // 4), F32)]
            + [vmem((2, D, FC), BF16), vmem((2, D, FC), BF16), vmem((2, FC, D), BF16)]
            + [vmem((49, D // 8, FC // 2), U32)] * 2 + [vmem((49, FC // 4, D // 4), U32)]
            + [dma((10,)), dma((11,)), dma((6,)), dma(()), pltpu.SMEM((1,), jnp.int32)]),
        compiler_params=pltpu.CompilerParams(
            vmem_limit_bytes=122 * 2 ** 20,
            flags={"XLA_TPU_EVENLY_DISTRIBUTE_CRITICAL_NODES": True},
        ),
    )(A_x.reshape(S, D), A_wqkv, A_wo, B_w_gate, B_w_up, B_w_down)
    return out.reshape(1, S, D)
```

```python
import functools

import jax
import jax.experimental.pallas as pl
import jax.experimental.pallas.tpu as pltpu
import jax.numpy as jnp
import numpy as np
from jax import lax

S, D, F = 2048, 1024, 3584
NH, DH, WIN, DIL = 32, 32, 8, 2
TM, FC = 512, 512
NT, NF = S // TM, F // FC
H, Q = TM // 2, TM // 4
NCB = D // 128
HALO = 16
PITCH = DH + 1
F32, BF16, U32 = jnp.float32, jnp.bfloat16, jnp.uint32
LOG2E = float(np.log2(np.e))
G0 = float(np.sqrt(2.0 / np.pi))
G1 = G0 * 0.044715
P = functools.partial

LHS = (((0, 1), (3, 1)), ((2, 1), (3, 1)), ((0, 1),), ((3, 1),), ((0, 1), (1, 1)), ((2, 1), (0, -1)), ((1, 1), (3, -1)))
RHS = (((0, 1), (3, 1)), ((0, 1),), ((1, 1), (3, -1)), ((2, 1), (0, -1)), ((3, 1),), ((0, 1), (1, 1)), ((2, 1), (3, 1)))
OUT = ({0: 1, 3: 1, 4: -1, 6: 1}, {2: 1, 4: 1}, {1: 1, 3: 1}, {0: 1, 1: -1, 2: 1, 5: 1})

ORDER = (1, 3, 2, 4, 0, 5, 6)
FFN_PLAN = ((0, 4, 6, 3, 1, 2, 5), (2, 5, 4, 3, 1, 6, 0))
FFN_PLAN_ODD = ((1, 3, 2, 4, 0, 5, 6), ())
FFN_PLAN_LAST = ((0, 1, 2, 5, 4, 3, 6), (3, 6, 1, 0, 4, 2, 5))

STEPS = ((0, 1, Q, 0, Q), (0, 1, Q, Q, H), (1, 0, H, 0, H), (1, 1, H, 0, H),
         (0, 2, H, 0, H), (1, 2, H, 0, H), (0, 3, H, 0, H), (1, 3, H, 0, H),
         (2, 0, H, 0, H), (2, 1, 64, 0, H), (2, 2, 64, 0, H), (2, 3, 64, 0, H),
         (3, 0, 64, 0, H), (3, 1, H, 0, H), (3, 2, H, 0, H), (3, 3, H, 0, H))
LN1_DONE = {-1: 1.5, 0: 2, 1: 2, 2: 3.5, 3: 3.75, 4: 4}
PROBS_DONE = {3: 0.6875, 4: 1.25, 5: 1.8125, 6: 2.4375, 7: 3, 8: 4}
MIX_DONE = {9: 1, 10: 2, 11: 3, 12: 4}
LN2_DONE = {13: 1, 14: 2, 15: 3}
FFN0_DONE = {9: 1, 10: 1.5, 11: 2.5, 12: 4}
WO_PARTS = {9: (0,), 10: (1, 2), 11: (3,)}


def _comb(terms, get):
    v = get(terms[0][0])
    for i, sign in terms[1:]:
        a, b = v.astype(F32), get(i).astype(F32)
        v = a + b if sign > 0 else a - b
    return v


def _collector(emit):
    part = {}

    def push(j, val):
        for q, terms in enumerate(OUT):
            if j not in terms:
                continue
            if q not in part:
                part[q] = (val, terms[j], 1)
                continue
            v, sign, n = part[q]
            v = v + val if sign == terms[j] else v - val if sign > 0 else val - v
            part[q] = (v, 1, n + 1)
            if n + 1 == len(terms):
                emit(q, v)
    return push


def _block(q1, q2):
    return 2 * (q1 // 2) + q2 // 2, 2 * (q1 % 2) + q2 % 2


def _cols(c, n=128):
    return pl.ds(c * n, n)


def _ds(start, n):
    return pl.ds(start if isinstance(start, int) else pl.multiple_of(start, n), n)


def _dot(a, b):
    return jnp.dot(pltpu.bitcast(a, BF16), pltpu.bitcast(b, BF16), preferred_element_type=F32)


def _put7(table, quads, dst, pair, col, base=0):
    quads = [q.astype(F32) for q in quads]
    v = jnp.concatenate([_comb(terms, lambda q: quads[q]) for terms in table], axis=0).reshape(7, -1, 128)
    dst[pl.ds(base, 7), _ds(pair, v.shape[1] // 2), _cols(col)] = pltpu.bitcast(v.astype(BF16), U32)


def _put49(table, get, dst, pair, col, j):
    quads = [_comb(table[j], lambda q1: get(*_block(q1, q2))) for q2 in range(4)]
    _put7(table, quads, dst, pair, col, 7 * j)


def _weave(main, n, sides, lead):
    done = [0] * len(sides)
    for k in range(n):
        next(main)
        for s, side in enumerate(sides):
            upto = min(len(side), -(-len(side) * (k + 1) // (n - lead)))
            for job in side[done[s]:upto]:
                job()
            done[s] = upto


def _span(fn, size, unit, done, k):
    if k not in done:
        return []
    lo, hi = (int(round(done.get(i, 0) * size / unit)) * unit for i in (k - 1, k))
    jobs = []
    for t in range(NT):
        a, b = max(lo - t * size, 0), min(hi - t * size, size)
        jobs += fn(t, a, b) if a < b else []
    return jobs


def _start(copies):
    for c in copies:
        c.start()


def _wait(copies):
    for c in copies:
        c.wait()


def _kernel(x_hbm, wqkv_hbm, wo_hbm, wg_hbm, wu_hbm, wd_hbm, o_hbm,
            xb, wraw, wp0, wp1, wp2, tmpa, tmpb, tmpc, xa, qb, kb, vb, ha, ab, acc,
            rg, ru, rd, gu0, gu1, dn, sx, sw, sf, so, go):
    wp = (wp0, wp1, wp2, wp0)
    gu = (gu0, gu1)
    copy = pltpu.make_async_copy

    def block(fn):
        pl.when(go[0] > 0)(fn)

    def cp_x_half(t, i):
        return [copy(x_hbm.at[pl.ds(r, Q)], xb.at[pl.ds(r, Q)], sx.at[r // Q])
                for r in (t * TM + i * Q, t * TM + H + i * Q)]

    def cp_x(t):
        return [copy(x_hbm.at[pl.ds(t * TM, TM)], xb.at[pl.ds(t * TM, TM)], sx.at[6 + t])]

    def cp_wq(i):
        return [copy(wqkv_hbm.at[pl.ds(r, 128), pl.ds(0, D)], wraw.at[0, pl.ds(r, 128)], sw.at[r // 128])
                for r in (i * 128, D // 2 + i * 128)]

    def cp_w(m):
        return [copy(wqkv_hbm.at[:, pl.ds(m * D, D)] if m < 3 else wo_hbm, wraw.at[m % 2], sw.at[7 + m])]

    def cp_up(c, s):
        return [copy(src.at[:, _ds(c * FC, FC)], dst.at[s], sf.at[3 * s + i])
                for i, (src, dst) in enumerate(((wg_hbm, rg), (wu_hbm, ru)))]

    def cp_down(c, s):
        return [copy(wd_hbm.at[_ds(c * FC, FC)], rd.at[s], sf.at[3 * s + 2])]

    def layernorm(load, parts, finish, lo, hi, lag):
        mu, xc, rs = {}, {}, {}

        def mean(*rows):
            for r in rows:
                mu[r] = jnp.sum(load(r).sum(0), axis=-1, keepdims=True) * (1.0 / D)

        def rstd(*rows):
            for r in rows:
                xc[r] = load(r) - mu[r]
                rs[r] = lax.rsqrt(jnp.sum((xc[r] * xc[r]).sum(0), axis=-1, keepdims=True) * (1.0 / D) + 1e-5)

        jobs = []
        for r in range(lo, hi + 2 * lag, 16):
            for fn, rr in ((mean, r), (rstd, r - lag)):
                if lo <= rr < hi:
                    jobs += [P(fn, rr + parts[i], rr + parts[i + 1]) for i in range(0, len(parts), 2)]
            if r - 2 * lag >= lo:
                jobs += finish(r - 2 * lag, lambda r, c: xc[r][c] * rs[r])
        return jobs

    def ln1(t, lo, hi):
        def load(r):
            return jnp.stack([xb[pl.ds(t * TM + r, 16), _cols(c)].astype(F32) for c in range(NCB)])

        def put(r, c, norm):
            _put7(LHS, [norm(r + q // 2 * H, q % 2 * 4 + c) for q in range(4)], xa.at[t], r // 2, c)
        return layernorm(load, (0, H), lambda r, norm: [P(put, r, c, norm) for c in range(4)], lo, hi, 16)

    def ln2(t, lo, hi):
        def load(r):
            return qb[:, pl.ds(t * TM + r, 16), :]

        def finish(r, norm):
            get = functools.cache(lambda c, i, k: norm(r + i * Q, 2 * k + c))
            return [P(_put49, LHS, P(get, c), ha.at[t], r // 2, c, j) for c in range(2) for j in range(7)]
        return layernorm(load, (0, Q, 2 * Q, 3 * Q), finish, lo, hi, 0)

    def prep_cols(m, i):
        tmp = (tmpa, tmpb)[i % 2]

        def fwd(c):
            w = jnp.concatenate([wraw[m % 2, pl.ds(b + i * 128, 128), _cols(c)] for b in (0, D // 2)], axis=0)
            wt = pltpu.bitcast(w, U32).T
            for h in range(4):
                tmp[pl.ds((4 * c + h) * PITCH, DH), :] = wt[h * DH:(h + 1) * DH]

        def back(c):
            rows = [tmp[pl.ds(4 * c + d, NH, stride=PITCH), :] for d in range(4)]
            tmpc[_cols(c), :] = jnp.concatenate(rows, axis=0).T

        def put(c, r0):
            for r in range(r0, r0 + 32, 8):
                quads = [tmpc[pl.ds((q % 2 * 4 + c) * 128 + q // 2 * 64 + r, 8), :] for q in range(4)]
                _put7(RHS, [pltpu.bitcast(v, BF16) for v in quads], wp[m], i * 64 + r, c)
        return ([P(fwd, c) for c in range(NCB)] + [P(back, c) for c in (0, 4, 1, 5, 2, 6, 3, 7)]
                + [P(put, c, r) for c in range(4) for r in (0, 32)])

    def prep_rows(i):
        def fwd(n, h0):
            for h in (h0, h0 + 1):
                w = wraw[1, pl.ds(h * DH, DH), _cols(4 * n + i)].astype(F32)
                (tmpa, tmpb)[n][pl.ds(h * PITCH, DH), :] = pltpu.bitcast(w, U32)

        def put(d):
            for h in (0, 16):
                quads = [(tmpa, tmpb)[q % 2][pl.ds(h * PITCH + q // 2 * 16 + d, 16, stride=PITCH), :]
                         for q in range(4)]
                _put7(RHS, [pltpu.bitcast(v, F32) for v in quads], wp[3], d * 16 + h // 2, i)
        return [P(fwd, n, h) for n in range(2) for h in range(0, NH, 2)] + [P(put, d) for d in range(16)]

    def prep_ffn(src, s, t, rows, cols, c, dst, pair, col):
        def get(r, k, n):
            return src[s, _ds(k * rows + t * (rows // NT) + r, 16), pl.ds(n * cols + c * 128, 128)]
        return [P(_put49, RHS, P(get, r), dst, pair + t * (rows // NT // 2) + r // 2, col, j)
                for r in range(0, rows // NT, 16) for j in range(7)]

    def prep_up(s, t):
        return sum((prep_ffn(src, s, t, D // 4, FC // 4, 0, gu[s], 0, i) for i, src in enumerate((rg, ru))), [])

    def prep_down(s, t):
        return sum((prep_ffn(rd, s, t, FC // 4, D // 4, c, dn, s * FC // 8, c) for c in range(2)), [])

    def probs(t, lo, hi):
        st = {}

        def dots(r, w):
            k = kb[:, pl.ds(t * TM + r + HALO - DIL * w, 8), :]
            for rr, ww in ((r, w), (r + 8, w + 8 // DIL)):
                if lo <= rr < hi:
                    st[rr, ww] = (qb[:, pl.ds(t * TM + rr, 8), :] * k).sum(0)

        def fold(r):
            l = jnp.concatenate([st[r, w] for w in range(WIN)], axis=0)
            st[r] = l + pltpu.roll(l, 64, 1)

        def softmax(r):
            l = (st[r] + pltpu.roll(st[r], 32, 1)) * (DH ** -0.5 * LOG2E)
            l = l.reshape(WIN, 8, 128)
            if t * TM + r < DIL * (WIN - 1):
                pos = t * TM + r + lax.broadcasted_iota(jnp.int32, l.shape, 1)
                l = jnp.where(pos >= DIL * lax.broadcasted_iota(jnp.int32, l.shape, 0), l, -1e9 * LOG2E)
            p = jnp.exp2(l - l.max(0))
            qb[:, pl.ds(t * TM + r, 8), :] = p * (1.0 / p.sum(0))

        jobs = [P(dots, lo - 8, w) for w in range(4)]
        for r in range(lo, hi, 8):
            jobs += [P(dots, r, w) for w in range(4)] + [P(fold, r)] + ([P(softmax, r - 8)] if r > lo else [])
        return jobs + [P(softmax, hi - 8)]

    def mix(t, lo, hi):
        st = {}

        def part(r, c, i):
            r0 = t * TM + i * H + r
            for w in range(WIN):
                pv = qb[w, pl.ds(r0, 16), :] * vb[pl.ds(2 * c, 2), pl.ds(r0 + HALO - DIL * w, 16), :]
                st[i] = st[i] + pv if w else pv
            if i:
                _put7(LHS, [st[q // 2][q % 2] for q in range(4)], xa.at[t], r // 2, c)
        return [P(part, r, c, i) for r in range(lo, hi, 16) for c in range(4) for i in range(2)]

    head, tail = prep_cols(0, 0), ln1(0, Q, H)
    for n, job in enumerate(head[2 * NCB:]):
        tail.insert(7 * n, job)
    go[0] = 1
    _start(cp_x_half(0, 0) + cp_wq(0))
    kb[:, pl.ds(0, HALO), :] = jnp.zeros((NCB, HALO, 128), F32)
    for now, later, jobs in ((cp_x_half(0, 0), cp_x_half(0, 1), ln1(0, 0, Q)),
                             (cp_wq(0), cp_wq(1), head[:2 * NCB]),
                             (cp_x_half(0, 1), cp_wq(2), tail)):
        _wait(now)
        _start(later)
        for job in jobs:
            job()

    def boot(i):
        if i == 0:
            _start(cp_wq(3))
            sides = [[lambda: None] * 6 + [lambda: _wait(cp_wq(1))] + prep_cols(0, 1)]
        elif i == 1:
            _wait(cp_wq(2))
            _start(cp_x_half(1, 0))
            sides = [prep_cols(0, 2)]
        elif i == 2:
            _wait(cp_wq(3) + cp_x_half(1, 0))
            _start(cp_x_half(1, 1))
            sides = [prep_cols(0, 3), ln1(1, 0, 48)]
        else:
            _start(cp_w(1))
            sides = [ln1(1, 48, Q)]

        def stages():
            for r in range(2):
                for n in range(2):
                    def emit(q, val):
                        for c in range(2):
                            qb[q % 2 * 4 + 2 * n + c, pl.ds(q // 2 * H + r * Q, Q), :] = val[:, c * 128:(c + 1) * 128]
                    push = _collector(emit)
                    for j in ORDER:
                        val = _dot(xa[0, j, _cols(r, Q // 2), _cols(i)], wp0[j, _cols(i, 64), _cols(n, 256)])
                        val = val + acc[2 * r + n, j] if i else val
                        if i < 3:
                            acc[2 * r + n, j] = val
                        else:
                            push(j, val)
                        yield
        _weave(stages(), 28, sides, 2)

    def step(k):
        m, t, rows, lo, hi = STEPS[k]
        prep = sum((prep_rows(i) for i in WO_PARTS.get(k, ())), [])
        if k == 0:
            _wait(cp_x_half(1, 1))
            _start(cp_x(2))
        elif k == 1:
            _wait(cp_w(1))
            _start(cp_x(3))
            prep = sum((prep_cols(1, i) for i in range(4)), [])
        elif k == 2:
            _wait(cp_x(2) + cp_x(3))
            _start(cp_w(2) + cp_up(0, 0) + cp_down(0, 0))
        elif k == 3:
            _start(cp_w(3))
        elif k == 4:
            _wait(cp_w(2))
            _start(cp_up(1, 1))
        elif k == 7:
            _wait(cp_w(3) + cp_up(0, 0) + cp_down(0, 0) + cp_up(1, 1))
        elif k == 9:
            vb[:, pl.ds(0, HALO), :] = jnp.broadcast_to(vb[:, pl.ds(HALO, 1), :], (NCB, HALO, 128))
        if 4 <= k < 8:
            prep = prep_cols(2, k - 4)
        sides = [_span(ln1, H, 16, LN1_DONE, k), _span(probs, TM, 8, PROBS_DONE, k), _span(mix, H, 16, MIX_DONE, k),
                 prep, _span(lambda t, a, b: (prep_up(0, t) + prep_down(0, t))[a:b], 84, 1, FFN0_DONE, k),
                 _span(ln2, Q, 16, LN2_DONE, k), prep_up(1, 0) if k == 11 else []]

        def stages():
            for n in range(4):
                for r in range(lo, hi, rows):
                    def emit(q, val):
                        r0, c = t * TM + q // 2 * H + r, q % 2 * 4 + n
                        if m == 0:
                            qb[c, pl.ds(r0, rows), :] = val
                        elif m == 1:
                            kb[c, pl.ds(HALO + r0, rows), :] = val
                        elif m == 2:
                            vb[2 * n + q % 2, pl.ds(HALO + r0, rows), :] = val
                        else:
                            qb[c, pl.ds(r0, rows), :] = val + xb[pl.ds(r0, rows), _cols(c)].astype(F32)
                    push = _collector(emit)
                    for j in ORDER:
                        push(j, _dot(xa[t, j, pl.ds(r // 2, rows // 2), :], wp[m][j, :, _cols(n)]))
                        yield
        _weave(stages(), 28 * ((hi - lo) // rows), sides, (hi - lo) // rows)

    for i in range(4):
        block(P(boot, i))
    for k in range(len(STEPS)):
        block(P(step, k))

    def ffn(s, t, side, first=False, last=False):
        act = {}

        def parked(i, n):
            return n, _ds(t * TM + i * Q, Q), slice(None)

        def geglu(q2, q1, val):
            g, u = val[:, :128], val[:, 128:]
            a = (g * u) * (jnp.tanh(g * (g * g * G1 + G0)) * 0.5 + 0.5)
            if s:
                kb[parked(*_block(q1, q2))] = a
            else:
                act[_block(q1, q2)] = a

        def store(q2, q1, val):
            i, n = _block(q1, q2)
            rows = _ds(t * TM + i * Q, Q)
            for c in range(2):
                xb[rows, _cols(2 * n + c)] = (qb[2 * n + c, rows, :] + val[:, c * 128:(c + 1) * 128]).astype(BF16)
            copy(xb.at[rows, _cols(n, 256)], o_hbm.at[rows, _cols(n, 256)], so).start()

        def down(j):
            if first:
                return _dot(ab[j, :, _cols(0)], dn[j, _cols(0, FC // 8), :])
            return acc[t, j] + _dot(ab[j], dn[j])

        def combine(j1, outer, product):
            inner = _collector(lambda q2, v: outer[q2](j1, v))
            for j2 in ORDER:
                inner(j2, product(7 * j1 + j2))
                yield

        def accumulate(j1):
            for j in range(7 * j1, 7 * j1 + 7):
                acc[t, j] = down(j)
                yield

        def stages():
            ups, downs = FFN_PLAN_LAST if last else FFN_PLAN_ODD if s else FFN_PLAN
            up = [_collector(P(geglu, q2)) for q2 in range(4)]
            out = [_collector(P(store, q2)) for q2 in range(4)]
            groups = [combine(j1, up, lambda j: _dot(ha[t, j], gu[s][j])) for j1 in ups]
            groups += [combine(j1, out, down) if last else accumulate(j1) for j1 in downs]
            for n, group in enumerate(groups):
                yield from group
                if 4 <= n < 11 and not s:
                    _put49(LHS, lambda i, k: act[i, k], ab, 0, 0, downs[n - 4])
                    if not first:
                        _put49(LHS, lambda i, k: kb[parked(i, k)], ab, 0, 1, downs[n - 4])
        _weave(stages(), 49 if s else 98, [side], 3)

    def tiles(fn, unroll=1):
        def body(i, _):
            for u in range(unroll):
                fn(i * unroll + u)
        lax.fori_loop(0, NT // unroll, body, None)

    def fetch(c):
        return cp_up(c + 1, 0) + cp_down(c, 1) + cp_down(c + 1, 0)

    def enter():
        _start(fetch(1))
        ffn(0, 0, ln2(NT - 1, 0, Q), first=True)

    def pair(p, _):
        c, more = 2 * p + 1, p < NF // 2 - 1
        _wait(fetch(c))
        pl.when(more)(lambda: _start(cp_up(c + 2, 1)))
        tiles(lambda t: ffn(1, t, prep_up(0, t) + prep_down(0, t) + prep_down(1, t)), 2)

        @pl.when(more)
        def _():
            _wait(cp_up(c + 2, 1))
            _start(fetch(c + 2))
            tiles(lambda t: ffn(0, t, prep_up(1, t)))

    block(enter)
    lax.fori_loop(1, NT, lambda t, _: ffn(0, t, prep_up(1, t), first=True), None)
    lax.fori_loop(0, NF // 2, pair, None)
    tiles(lambda t: ffn(0, t, [], last=True))
    copy(xb, o_hbm, so).wait()


@jax.jit
def pallas_sequential_preLN__sliding_local_dilated__glu_gated_geglu__prompt_kernel(
    A_x: jax.Array,
    A_wqkv: jax.Array,
    A_wo: jax.Array,
    B_x: jax.Array,
    B_w_gate: jax.Array,
    B_w_up: jax.Array,
    B_w_down: jax.Array,
):
    del B_x
    hbm = pl.BlockSpec(memory_space=pl.ANY)
    vmem, dma = pltpu.VMEM, pltpu.SemaphoreType.DMA
    out = pl.pallas_call(
        _kernel,
        in_specs=[hbm] * 6,
        out_specs=hbm,
        out_shape=jax.ShapeDtypeStruct((S, D), BF16),
        scratch_shapes=(
            [vmem((S, D), BF16), vmem((2, D, D), BF16)] + [vmem((7, D // 4, D // 2), U32)] * 3
            + [vmem((NH * PITCH + DH, 128), U32)] * 2 + [vmem((D, 128), U32), vmem((NT, 7, H // 2, D // 2), U32)]
            + [vmem((NCB, S, 128), F32)] + [vmem((NCB, HALO + S, 128), F32)] * 2
            + [vmem((NT, 49, Q // 2, D // 4), U32), vmem((49, Q // 2, FC // 2), U32), vmem((NT, 49, Q, D // 4), F32)]
            + [vmem((2, D, FC), BF16), vmem((2, D, FC), BF16), vmem((2, FC, D), BF16)]
            + [vmem((49, D // 8, FC // 2), U32)] * 2 + [vmem((49, FC // 4, D // 4), U32)]
            + [dma((10,)), dma((11,)), dma((6,)), dma(()), pltpu.SMEM((1,), jnp.int32)]),
        compiler_params=pltpu.CompilerParams(
            vmem_limit_bytes=122 * 2 ** 20,
            flags={"XLA_TPU_EVENLY_DISTRIBUTE_CRITICAL_NODES": True},
        ),
    )(A_x.reshape(S, D), A_wqkv, A_wo, B_w_gate, B_w_up, B_w_down)
    return out.reshape(1, S, D)
```
